```python
import os as _os
_os.environ.setdefault('JAX_PLATFORMS', 'cpu')
import jax
import jax.numpy as jnp

def _softmax(x, axis=-1):
    return jax.nn.softmax(x, axis=axis)

def _gelu(x):
    return jax.nn.gelu(x, approximate=True)

def _silu(x):
    return jax.nn.silu(x)

def _sigmoid(x):
    return jax.nn.sigmoid(x)

def _layernorm(x, axis=-1, eps=1e-05):
    m = jnp.mean(x, axis=axis, keepdims=True)
    v = jnp.var(x, axis=axis, keepdims=True)
    return (x - m) / jnp.sqrt(v + eps)

def _scatter_add(tgt, idx, src, axis=0):
    return tgt.at[idx].add(src)

def _segment_sum(src, seg, n):
    return jax.ops.segment_sum(src, seg, n)

class _Rng:

    def __init__(self, key):
        self._k = key

    def _next(self):
        self._k, sub = jax.random.split(self._k)
        return sub

    def normal(self, shape):
        return jax.random.normal(self._next(), shape, dtype=jnp.bfloat16)

    def randint(self, lo, hi, shape):
        return jax.random.randint(self._next(), shape, lo, hi, dtype=jnp.int32)

    def uniform(self, shape, lo=0.0, hi=1.0):
        return jax.random.uniform(self._next(), shape, jnp.bfloat16, lo, hi)

    def permutation(self, n):
        return jax.random.permutation(self._next(), n)
kernel_name = 'recurrent_scan__memory_aug_recurrent_mem_tr__mixer_gmlp__prompt'

def setup_inputs():
    _rng = _Rng(jax.random.key(int.from_bytes(__import__("os").urandom(4), "little")))
    _w = lambda a: (lambda t: t.astype(jnp.bfloat16) if jnp.issubdtype(t.dtype, jnp.floating) else t)(jnp.asarray(a))

    def _A_setup():
        B, S, Dm = (1, 2048, 640)
        H, Dh = (32, 128)
        M, seg = (8, 32)
        seg = min(seg, S)
        S = S // seg * seg
        return {'x': _w((lambda *s: _rng.normal(s) * 0.05)(B, S, Dm)), 'mem0': _w((lambda *s: _rng.normal(s) * 0.1)(B, M, Dm)), 'Wq': _w((lambda *s: _rng.normal(s) * 1.6)(Dm, H, Dh) * Dm ** (-0.5)), 'Wk': _w((lambda *s: _rng.normal(s) * 1.6)(Dm, H, Dh) * Dm ** (-0.5)), 'Wv': _w((lambda *s: _rng.normal(s) * 0.1)(Dm, H, Dh) * Dm ** (-0.5)), 'Wo': _w((lambda *s: _rng.normal(s) * 0.1)(H, Dh, Dm) * (H * Dh) ** (-0.5)), 'seg_len': seg}
    _A_in = _A_setup()

    def _B_setup():
        B, S, D, F = (1, 2048, 640, 1728)
        Fh = F // 2
        return {'x': _w((lambda *s: _rng.normal(s) * 0.05)(B, S, D)), 'w_in': _w((lambda *s: _rng.normal(s) * 0.8)(D, 2 * Fh)), 'w_sp': _w(0.01 * (lambda *s: _rng.normal(s) * 0.8)(S, S)), 'b_sp': _w(1.0 + 0.01 * (lambda *s: _rng.normal(s) * 0.05)(S)), 'w_out': _w((lambda *s: _rng.normal(s) * 0.05)(Fh, D))}
    _B_in = _B_setup()
    return {'A_x': _A_in['x'], 'A_mem0': _A_in['mem0'], 'A_Wq': _A_in['Wq'], 'A_Wk': _A_in['Wk'], 'A_Wv': _A_in['Wv'], 'A_Wo': _A_in['Wo'], 'A_seg_len': _A_in['seg_len'], 'B_x': _B_in['x'], 'B_w_in': _B_in['w_in'], 'B_w_sp': _B_in['w_sp'], 'B_b_sp': _B_in['b_sp'], 'B_w_out': _B_in['w_out']}

def reference(A_x, A_mem0, A_Wq, A_Wk, A_Wv, A_Wo, A_seg_len, B_x, B_w_in, B_w_sp, B_b_sp, B_w_out):

    def _A_ref(x, mem0, Wq, Wk, Wv, Wo, seg_len):
        B, S, Dm = x.shape
        H, Dh = (Wq.shape[1], Wq.shape[2])
        M = mem0.shape[1]
        scale = Dh ** (-0.5)
        n_seg = S // seg_len
        L = M + seg_len
        idx = jnp.arange(L)
        mask = (idx[:, None] < M) | (idx[:, None] >= idx[None, :])
        mem = mem0
        outs = []
        for s in range(n_seg):
            xs = x[:, s * seg_len:(s + 1) * seg_len, :].copy()
            h = jnp.concatenate([mem, xs], axis=1)
            q = jnp.einsum('btd,dhe->bhte', h, Wq)
            k = jnp.einsum('btd,dhe->bhte', h, Wk)
            v = jnp.einsum('btd,dhe->bhte', h, Wv)
            scores = jnp.einsum('bhqe,bhke->bhqk', q, k) * scale
            scores = jnp.where(mask[None, None], scores, -1000000000.0)
            p = _softmax(scores, axis=-1)
            o = jnp.einsum('bhqk,bhke->bhqe', p, v)
            o = jnp.einsum('bhte,hed->btd', o, Wo)
            mem = o[:, :M, :].copy()
            outs.append(o[:, M:, :])
        return jnp.concatenate(outs, axis=1)

    def _B_ref(x, w_in, w_sp, b_sp, w_out):
        B, S, D = x.shape
        F = w_in.shape[-1]
        Fh = F // 2
        z = _gelu(jnp.einsum('bsd,df->bsf', x, w_in))
        z1 = z[..., :Fh].copy()
        z2 = _layernorm(z[..., Fh:], axis=-1)
        g = jnp.einsum('ts,bsf->btf', w_sp, z2) + b_sp[None, :, None]
        return jnp.einsum('bsf,fd->bsd', z1 * g, w_out)
    x = A_x
    xn = _layernorm(x, axis=-1)
    s = _A_ref(xn, A_mem0, A_Wq, A_Wk, A_Wv, A_Wo, A_seg_len)
    g = _silu(_B_ref(xn, B_w_in, B_w_sp, B_b_sp, B_w_out))
    return x + s * g
```

```python
import functools, math
import jax
import jax.numpy as jnp
import jax.experimental.pallas as pl
import jax.experimental.pallas.tpu as pltpu

F32 = jnp.float32
BF16 = jnp.bfloat16
U32 = jnp.uint32
D1, D2, D3 = 1, 2, 3
RPAD = 4


def _ln(x, eps=1e-5):
    m = jnp.mean(x, axis=-1, keepdims=True)
    xc = x - m
    v = jnp.mean(xc * xc, axis=-1, keepdims=True)
    return xc * jax.lax.rsqrt(v + eps)


def _dot_t(a, b):
    return jax.lax.dot_general(a, b, (((1,), (1,)), ((), ())), preferred_element_type=F32)


def _kernel(x_hbm, mem0_ref, wq_hbm, wk_hbm, wv_hbm, wo_hbm, win_hbm, wsp_ref, b_ref, wout_hbm,
            o_ref,
            x_ref, xn_ref, z1_ref, z2_ref, mem_ref, wraw_ref, w_ref, wo_ref, win_ref, wout_ref,
            btab_ref, sems, *, S, D, H, Dh, M, SEG, FH, PC):
    j = pl.program_id(0)
    L = M + SEG
    NP = H // 2
    DH2 = D // 2
    RS = DH2 + RPAD
    NC = S // PC
    HR = D * H // 2

    def x_copy(c):
        return pltpu.make_async_copy(x_hbm.at[0, pl.ds(c * PC, PC), :], x_ref.at[pl.ds(c * PC, PC), :], sems.at[c])

    def w_copy(hh):
        src = (wq_hbm, wk_hbm, wv_hbm)[hh // 2]
        return pltpu.make_async_copy(src.at[pl.ds((hh % 2) * HR, HR), :], wraw_ref.at[hh], sems.at[NC + hh])

    win_copy = pltpu.make_async_copy(win_hbm, win_ref, sems.at[NC + 6])
    wo_copy = pltpu.make_async_copy(wo_hbm, wo_ref, sems.at[NC + 7])
    wout_copy = pltpu.make_async_copy(wout_hbm, wout_ref, sems.at[NC + 8])

    @pl.when(j == 0)
    def _prologue():
        x_copy(0).start()
        win_copy.start()
        for c in range(1, NC):
            x_copy(c).start()
        for hh in range(6):
            w_copy(hh).start()
        wo_copy.start()
        wout_copy.start()

        mem_ref[...] = mem0_ref[0].astype(F32)
        bt = jnp.transpose(jnp.concatenate([b_ref[...].astype(F32)] * 8, axis=0))
        for i in range(S // 128):
            btab_ref[i * 128:(i + 1) * 128, :] = jnp.broadcast_to(bt[:, i:i + 1], (128, 128))

        def ln_chunk(r):
            xn_ref[pl.ds(r, PC), :] = _ln(x_ref[pl.ds(r, PC), :].astype(F32))

        def z_chunk(r):
            xnb = xn_ref[pl.ds(r, PC), :].astype(BF16)
            z2 = jax.nn.gelu(_dot_t(xnb, win_ref[FH:, :]), approximate=True)
            z2_ref[pl.ds(r, PC), :] = _ln(z2).astype(BF16)
            z1 = jax.nn.gelu(_dot_t(xnb, win_ref[:FH, :]), approximate=True)
            z1_ref[pl.ds(r, PC), :] = z1.astype(BF16)

        def relayout(hh):
            base = (hh // 2) * (H * RS) + (hh % 2) * (DH2 // 2)
            G = 8
            for g in range(DH2 // 2 // G):
                blk = pltpu.bitcast(wraw_ref[hh, g * G * 2 * H:(g + 1) * G * 2 * H, :], U32)
                for u in range(G):
                    a = blk[u * H:u * H + NP]
                    b = blk[u * H + NP:(u + 1) * H]
                    lo = (a & jnp.uint32(0xFFFF)) | (b << 16)
                    hi = (a >> 16) | (b & jnp.uint32(0xFFFF0000))
                    w_ref[pl.ds(base + g * G + u, NP, stride=RS), :] = lo
                    w_ref[pl.ds(base + NP * RS + g * G + u, NP, stride=RS), :] = hi

        x_copy(0).wait()
        ln_chunk(0)
        win_copy.wait()
        for c in range(2):
            x_copy(c + 1).wait()
            ln_chunk((c + 1) * PC)
            z_chunk(c * PC)
        for c in range(3, NC):
            x_copy(c).wait()

        def body(c, carry):
            hh = c - 2
            pltpu.make_async_copy(wq_hbm.at[pl.ds(0, HR), :], wraw_ref.at[hh], sems.at[NC + hh]).wait()
            r = pl.multiple_of(c * PC, PC)
            rn = pl.multiple_of(jnp.minimum(c + 1, NC - 1) * PC, PC)
            z_chunk(r)
            ln_chunk(rn)
            relayout(hh)
            return carry
        jax.lax.fori_loop(2, NC, body, 0)
        wo_copy.wait()
        wout_copy.wait()

    scale = Dh ** -0.5
    c_exp = scale * math.log2(math.e)
    row = jax.lax.broadcasted_iota(jnp.int32, (2 * L, 2 * L), 0)
    col = jax.lax.broadcasted_iota(jnp.int32, (2 * L, 2 * L), 1)
    rhi = row >= L
    chi = col >= L
    rl = jnp.where(rhi, row - L, row)
    cl = jnp.where(chi, col - L, col)
    same = rhi == chi
    causal = (rl < M) | (rl >= cl)
    valid = same & causal
    fill = jnp.where(same, -1e9 / scale, -jnp.inf).astype(F32)

    def wpair(p):
        parts = []
        for w in range(3):
            for par in range(2):
                s = (w * H + par * NP + p) * RS
                parts.append(pltpu.bitcast(w_ref[s:s + DH2, :], BF16))
        return jnp.concatenate(parts, axis=1)

    def stack(qkv, i):
        return jnp.concatenate([qkv[:, i * Dh:(i + 1) * Dh], qkv[:, (i + 1) * Dh:(i + 2) * Dh]], axis=0).astype(BF16)

    def scores(q2, k2):
        s = jax.lax.dot_general(q2, k2, (((1,), (1,)), ((), ())), preferred_element_type=F32)
        s = jnp.where(valid, s, fill)
        m = jnp.max(s, axis=-1, keepdims=True)
        e = jnp.exp2((s - m) * c_exp)
        l = jnp.sum(e, axis=-1, keepdims=True)
        return e.astype(BF16), 1.0 / l

    def pv(e, rl_, v2):
        o2 = jnp.dot(e, v2, preferred_element_type=F32) * rl_
        return jnp.concatenate([o2[:L], o2[L:]], axis=1)

    r0 = pl.multiple_of(j * (2 * SEG), 2 * SEG)
    xn = xn_ref[pl.ds(r0, 2 * SEG), :]
    mem = mem_ref[...]

    wsp = wsp_ref[...]
    bcol = btab_ref[pl.ds(r0, 2 * SEG), :]
    tparts = []
    edges = list(range(0, FH, 128)) + [FH]

    def gcol(c):
        lo, hi = edges[c], edges[c + 1]
        g = jnp.dot(wsp, z2_ref[:, lo:hi], preferred_element_type=F32) + bcol[:, :hi - lo]
        tparts.append((z1_ref[pl.ds(r0, 2 * SEG), lo:hi].astype(F32) * g).astype(BF16))

    res = {}

    def gout():
        t = jnp.concatenate(tparts, axis=1)
        u = jnp.dot(t, wout_ref[...], preferred_element_type=F32)
        res["gate"] = u * jax.nn.sigmoid(u)

    def run_step(h, post_proj, pre_o, fillers):
        qkv, sm, oo = {}, {}, {}
        acc = None
        fillers = list(fillers)
        for t in range(NP + D3):
            if t < NP:
                r = jnp.dot(h, wpair(t), preferred_element_type=F32)
                r = post_proj(t, r)
                qkv[t] = (stack(r, 0), stack(r, 2), stack(r, 4))
            else:
                fillers.pop(0)()
            p = t - D1
            if 0 <= p < NP:
                sm[p] = scores(qkv[p][0], qkv[p][1])
            p = t - D2
            if 0 <= p < NP:
                oo[p] = pre_o(p, pv(sm[p][0], sm[p][1], qkv[p][2])).astype(BF16)
            p = t - D3
            if 0 <= p < NP:
                tt = jnp.dot(oo[p], wo_ref[p * 2 * Dh:(p + 1) * 2 * Dh, :], preferred_element_type=F32)
                acc = tt if acc is None else acc + tt
        for f in fillers:
            f()
        return acc

    stash_qkv, stash_o = {}, {}

    def postA(t, r):
        stash_qkv[t] = r[L:]
        return r[:L]

    def preA(p, o):
        stash_o[p] = o[SEG:]
        return o[:SEG]

    hA = jnp.concatenate([mem, xn[:SEG + M]], axis=0).astype(BF16)
    accA = run_step(hA, postA, preA, [functools.partial(gcol, c) for c in range(4)])
    hB = jnp.concatenate([accA[:M], xn[SEG + M:]], axis=0).astype(BF16)
    accB = run_step(hB, lambda t, r: jnp.concatenate([r[:M], stash_qkv[t], r[M:]], axis=0),
                    lambda p, o: jnp.concatenate([o, stash_o[p]], axis=0),
                    [functools.partial(gcol, c) for c in range(4, 7)] + [gout])
    mem_ref[...] = accB[:M]
    s_out = jnp.concatenate([accA[M:], accB[L:], accB[M:L]], axis=0)
    xr = x_ref[pl.ds(r0, 2 * SEG), :].astype(F32)
    o_ref[0] = (xr + s_out * res["gate"]).astype(o_ref.dtype)


@functools.partial(jax.jit, static_argnames=("A_seg_len",))
def pallas_recurrent_scan__memory_aug_recurrent_mem_tr__mixer_gmlp__prompt_kernel(A_x, A_mem0, A_Wq, A_Wk, A_Wv, A_Wo, A_seg_len, B_x, B_w_in, B_w_sp, B_b_sp, B_w_out):
    _, S, D = A_x.shape
    H, Dh = A_Wq.shape[1], A_Wq.shape[2]
    M = A_mem0.shape[1]
    SEG = int(A_seg_len)
    FH = B_w_in.shape[1] // 2
    PC = 256
    wq, wk, wv = (w.reshape(D * H, Dh) for w in (A_Wq, A_Wk, A_Wv))
    wo = A_Wo.reshape(H * Dh, D)
    b = B_b_sp.reshape(S // 128, 128)
    win_t = B_w_in.T
    R = 2 * SEG
    kern = functools.partial(_kernel, S=S, D=D, H=H, Dh=Dh, M=M, SEG=SEG, FH=FH, PC=PC)
    full = lambda a: pl.BlockSpec(a.shape, lambda j: (0,) * a.ndim)
    anyspec = pl.BlockSpec(memory_space=pl.ANY)
    return pl.pallas_call(
        kern,
        grid=(S // R,),
        in_specs=[anyspec, full(A_mem0), anyspec, anyspec, anyspec, anyspec, anyspec,
                  pl.BlockSpec((R, S), lambda j: (j, 0)),
                  full(b), anyspec],
        out_specs=pl.BlockSpec((1, R, D), lambda j: (0, j, 0)),
        out_shape=jax.ShapeDtypeStruct(A_x.shape, A_x.dtype),
        scratch_shapes=[
            pltpu.VMEM((S, D), BF16),
            pltpu.VMEM((S, D), F32),
            pltpu.VMEM((S, FH), BF16),
            pltpu.VMEM((S, FH), BF16),
            pltpu.VMEM((M, D), F32),
            pltpu.VMEM((6, D * H // 2, Dh), BF16),
            pltpu.VMEM((3 * H * (D // 2 + RPAD), Dh), U32),
            pltpu.VMEM(wo.shape, BF16),
            pltpu.VMEM(win_t.shape, BF16),
            pltpu.VMEM(B_w_out.shape, BF16),
            pltpu.VMEM((S, 128), F32),
            pltpu.SemaphoreType.DMA((S // PC + 9,)),
        ],
        compiler_params=pltpu.CompilerParams(dimension_semantics=("arbitrary",), vmem_limit_bytes=110 * 1024 * 1024),
    )(A_x, A_mem0, wq, wk, wv, wo, win_t, B_w_sp, b, B_w_out)
```

```python
import functools
import math

import jax
import jax.numpy as jnp
import jax.experimental.pallas as pl
import jax.experimental.pallas.tpu as pltpu

F32 = jnp.float32
BF16 = jnp.bfloat16
U32 = jnp.uint32

RPAD = 4
UNR = 2
SB = 128
ZU = 4
PG = 8
NCH = 4
NCAR = 2
GRID = None
INTERPRET = False


def _ln(x, eps=1e-5):
    m = jnp.mean(x, axis=-1, keepdims=True)
    xc = x - m
    v = jnp.mean(xc * xc, axis=-1, keepdims=True)
    return xc * jax.lax.rsqrt(v + eps)


def _dot(a, b):
    return jnp.dot(a, b, preferred_element_type=F32)


def _dot_t(a, b):
    return jax.lax.dot_general(a, b, (((1,), (1,)), ((), ())), preferred_element_type=F32)


def _bf(u):
    return pltpu.bitcast(u, BF16)


def _pk(x):
    return pltpu.bitcast(x, U32)


def _gelu(x):
    c0 = math.sqrt(2.0 / math.pi)
    u = x * (x * x * (c0 * 0.044715) + c0)
    h = 0.5 * x
    return h * jnp.tanh(u) + h


def _mult(i, k):
    return i if isinstance(i, int) else pl.multiple_of(i, k)


def _kernel(x_hbm, mem0_hbm, wq_hbm, wk_hbm, wv_hbm, wo_hbm, win_hbm, wsp_hbm, b_hbm, wout_hbm,
            o_hbm,
            x_ref, xn_ref, xs_ref, wq_ref, wkv_ref, z2_ref, mem0_ref, wraw_ref, wo_ref, win_ref,
            wsp_ref, wout_ref, b_ref, btab_ref, o_ref, sems,
            *, S, D, H, Dh, M, SEG, FH):
    L = M + SEG
    R = 2 * SEG
    RU = R * UNR
    NIT = S // RU
    NP = H // 2
    HG = NP // 2
    DH2 = D // 2
    RS = DH2 + RPAD
    QL = SEG - M
    NS = S // R * 2 * M
    NX = SB // R * 2 * M
    edges = list(range(0, FH, 128)) + [FH]
    NT = len(edges) - 1
    NB = S // SB
    NZ = NB // ZU
    ZOFF = H * RS
    QOFF = 2 * H * RS
    WQP = D * H // NZ

    sem_ids = iter(range(sems.shape[0]))

    def sem_block(n):
        return [next(sem_ids) for _ in range(n)][0]

    def rows_copy(src, dst, lo, n, sem):
        return pltpu.make_async_copy(src.at[pl.ds(lo, n), :], dst.at[pl.ds(lo, n), :], sems.at[sem])

    def full_copy(src, dst):
        return pltpu.make_async_copy(src, dst, sems.at[sem_block(1)])

    x2 = x_hbm.at[0]
    xa_copy = rows_copy(x2, x_ref, 0, 2 * SB, sem_block(1))
    xb_copy = rows_copy(x2, x_ref, 2 * SB, (ZU - 1) * SB, sem_block(1))
    xc_copy = rows_copy(x2, x_ref, (ZU + 1) * SB, ZU * SB, sem_block(1))
    xd_copy = rows_copy(x2, x_ref, (2 * ZU + 1) * SB, S - (2 * ZU + 1) * SB, sem_block(1))
    win1_copy = rows_copy(win_hbm, win_ref, 0, FH, sem_block(1))
    win2_copy = rows_copy(win_hbm, win_ref, FH, FH, sem_block(1))
    wk_copy = full_copy(wk_hbm, wraw_ref.at[1])
    wv_copy = full_copy(wv_hbm, wraw_ref.at[2])
    wo_copy = full_copy(wo_hbm, wo_ref)
    wout_copy = full_copy(wout_hbm, wout_ref)
    mem0_copy = full_copy(mem0_hbm, mem0_ref)
    b_copy = full_copy(b_hbm, b_ref)
    wq_sem, wsp_sem, out_sem = sem_block(NZ), sem_block(NIT), sem_block(NIT)

    def wq_copy(c):
        return rows_copy(wq_hbm, wraw_ref.at[0], c * WQP, WQP, wq_sem + c)

    def wsp_copy(i):
        return rows_copy(wsp_hbm, wsp_ref, i * RU, RU, wsp_sem + i)

    def out_copy(i):
        return rows_copy(o_ref, o_hbm.at[0], i * RU, RU, out_sem + i)

    for c in ([xa_copy, win1_copy, b_copy, mem0_copy, win2_copy, xb_copy, xc_copy, wq_copy(0), wq_copy(1), xd_copy]
              + [wq_copy(c) for c in range(2, NZ)] + [wk_copy, wv_copy, wo_copy, wout_copy]
              + [wsp_copy(i) for i in range(NIT)]):
        c.start()

    def wdst(w):
        return (wq_ref, 0) if isinstance(w, int) and w == 0 else (wkv_ref, (w - 1) * H)

    def wpair(ws, p):
        parts = []
        for w in ws:
            ref, h0 = wdst(w)
            for par in range(2):
                parts.append(_bf(ref[pl.ds((h0 + par * NP + p) * RS, DH2), :]))
        return jnp.concatenate(parts, axis=1)

    def relayout(w, grp, j0, nj):
        src = wraw_ref.at[w, pl.ds(pl.multiple_of((j0 * H + grp * HG) * 2, HG * 2), (nj * H - HG) * 2), :]
        dst, h0 = wdst(w)
        base = (h0 + grp * HG) * RS + j0
        for u in range(nj):
            a = _pk(src[u * H * 2:(u * H + HG) * 2, :])
            b = _pk(src[(u * H + NP) * 2:(u * H + NP + HG) * 2, :])
            dst[pl.ds(base + u, HG, stride=RS), :] = (a & jnp.uint32(0xFFFF)) | (b << 16)
            dst[pl.ds(base + NP * RS + u, HG, stride=RS), :] = (a >> 16) | (b & jnp.uint32(0xFFFF0000))

    class Blk:
        def __init__(self, i0, n):
            v = lambda ref, k: ref.at[pl.ds(_mult(i0 * k, k), n * k), :]
            self.x, self.xn, self.xs, self.z2 = v(x_ref, SB), v(xn_ref, SB // 2), v(xs_ref, NX), v(z2_ref, SB // 2)
            self.i0 = i0

        def ln(self, s):
            xn = _ln(self.x[s * SB:(s + 1) * SB, :].astype(F32))
            xb = xn.astype(BF16)
            self.xn[s * SB // 2:(s + 1) * SB // 2, :] = _pk(xb)
            sel = jnp.concatenate([xn[k * R + QL:k * R + QL + 2 * M] for k in range(SB // R)], axis=0)
            self.xs[s * NX:(s + 1) * NX, :] = sel.astype(BF16)
            return xb

        def z2_rows(self, s, xb):
            z2 = _ln(_gelu(_dot_t(xb, win_ref[FH:, :])))
            self.z2[s * SB // 2:(s + 1) * SB // 2, :] = _pk(z2.astype(BF16))

        def z1_rows(self, s, xb, extra=None):
            z1 = _dot_t(xb, win_ref[:FH, :])
            r = (self.i0 + s) * (SB // 2)
            for c in range(NT):
                wq_ref[pl.ds(_mult(ZOFF + c * (S // 2) + r, 8), SB // 2), :edges[c + 1] - edges[c]] = (
                    _pk(z1[:, edges[c]:edges[c + 1]].astype(BF16)))
                if extra is not None:
                    extra(c)

    blk0 = Blk(0, ZU + 1)
    xa_copy.wait()
    xb0 = blk0.ln(0)
    xb1 = blk0.ln(1)
    b_copy.wait()
    bt = jnp.transpose(jnp.concatenate([b_ref[...].astype(F32)] * (128 * 128 // S), axis=0))
    for i in range(S // 128):
        btab_ref[i * 128:(i + 1) * 128, :] = jnp.broadcast_to(bt[:, i:i + 1], (128, 128))
    win1_copy.wait()
    blk0.z1_rows(0, xb0)
    blk0.z1_rows(1, xb1)
    win2_copy.wait()
    xb_copy.wait()
    blk0.z2_rows(0, xb0)
    xb = blk0.ln(2)
    blk0.z2_rows(1, xb1)
    for i in range(2, ZU):
        nxt = blk0.ln(i + 1)
        blk0.z2_rows(i, xb)
        blk0.z1_rows(i, xb)
        xb = nxt
    xc_copy.wait()
    wq_copy(0).wait()
    CJ = -(-DH2 // ((NZ - 1) * ZU * NT))

    def zgroup(c, xb):
        wq_copy(c).wait()

        @pl.when(c == 2)
        def _():
            xd_copy.wait()

        blk = Blk(c * ZU, ZU)
        for s in range(ZU):
            def extra(t):
                j0 = jnp.minimum((((c - 1) * ZU + s) * NT + t) * CJ, DH2 - CJ)
                relayout(0, 0, j0, CJ)
                relayout(0, 1, j0, CJ)

            if s + 1 < ZU:
                nxt = blk.ln(s + 1)
            else:
                nxt = Blk(jnp.minimum((c + 1) * ZU, NB - 1), 1).ln(0)
            if s == 0:
                blk.z1_rows(s, xb, extra)
            blk.z2_rows(s, xb)
            if s > 0:
                blk.z1_rows(s, xb, extra)
            xb = nxt
        return xb
    jax.lax.fori_loop(1, NZ, zgroup, xb)

    wk_copy.wait()
    wv_copy.wait()
    UPP = NP // 4
    NJ = DH2 // UPP

    def qpre(i, carry):
        xs = xs_ref[...]
        nr = NS // NCH
        nj = NJ // (2 * NCH)
        for k in range(PG):
            p = i * PG + k
            unit = p // UPP
            q = _dot(xs, wpair((0,), p))
            for par in range(2):
                for c in range(NCH):
                    wkv_ref[pl.ds(pl.multiple_of(QOFF + (2 * p + par) * NS + c * nr, 8), nr), :] = _pk(
                        q[c * nr:(c + 1) * nr, par * Dh:(par + 1) * Dh])
                    relayout(1 + unit // 2, unit % 2, (p % UPP) * NJ + (par * NCH + c) * nj, nj)
        return carry
    jax.lax.fori_loop(0, NP // PG, qpre, 0)

    def qpre_rows(p, r):
        return jnp.concatenate(
            [pltpu.bitcast(wkv_ref[pl.ds(pl.multiple_of(QOFF + (2 * p + par) * NS + r, 8), M), :], F32)
             for par in range(2)], axis=1)

    def gcol(jj, c):
        r0 = _mult(jj * R, R)
        w = edges[c + 1] - edges[c]
        g = _dot(wsp_ref[pl.ds(r0, R), :], _bf(z2_ref[:, edges[c]:edges[c + 1]])) + btab_ref[pl.ds(r0, R), :w]
        z1 = _bf(wq_ref[pl.ds(_mult(ZOFF + c * (S // 2) + jj * SEG, 8), SEG), :w]).astype(F32)
        return (_gelu(z1) * g).astype(BF16)

    wo_copy.wait()
    wout_copy.wait()
    mem0_copy.wait()
    wsp_copy(0).wait()
    t_init = tuple(gcol(0, c) for c in range(NCAR))

    scale = Dh ** -0.5
    c_exp = scale * math.log2(math.e)

    def main(it, carry):
        @pl.when(it + 1 < NIT)
        def _():
            wsp_copy(it + 1).wait()

        row = jax.lax.broadcasted_iota(jnp.int32, (2 * L, 2 * L), 0)
        col = jax.lax.broadcasted_iota(jnp.int32, (2 * L, 2 * L), 1)
        rhi = row >= L
        chi = col >= L
        rl = jnp.where(rhi, row - L, row)
        cl = jnp.where(chi, col - L, col)
        same = rhi == chi
        valid = same & ((rl < M) | (rl >= cl))
        fill = jnp.where(same, -1e9 / scale, -jnp.inf).astype(F32)

        def stack(a, i):
            return jnp.concatenate([a[:, i * Dh:(i + 1) * Dh], a[:, (i + 1) * Dh:(i + 2) * Dh]], axis=0).astype(BF16)

        def scores(q2, k2):
            s = jnp.where(valid, _dot_t(q2, k2), fill)
            m = jnp.max(s, axis=-1, keepdims=True)
            e = jnp.exp2((s - m) * c_exp)
            l = jnp.sum(e, axis=-1, keepdims=True)
            return e.astype(BF16), 1.0 / l

        def pv(e, inv_l, v2):
            o2 = _dot(e, v2) * inv_l
            return jnp.concatenate([o2[:L], o2[L:]], axis=1)

        def run_step(proj, pre_o, fillers):
            qkv, sm, oo = {}, {}, {}
            acc = None
            for t in range(NP + 3):
                if t < NP:
                    qkv[t] = proj(t)
                else:
                    fillers[t - NP]()
                p = t - 3
                if 0 <= p < NP:
                    tt = _dot(oo[p], wo_ref[p * 2 * Dh:(p + 1) * 2 * Dh, :])
                    acc = tt if acc is None else acc + tt
                p = t - 1
                if 0 <= p < NP:
                    sm[p] = scores(qkv[p][0], qkv[p][1])
                p = t - 2
                if 0 <= p < NP:
                    oo[p] = pre_o(p, pv(sm[p][0], sm[p][1], qkv[p][2])).astype(BF16)
            fillers[3]()
            return acc

        def pair_step(jj, mem, tcar):
            r0 = pl.multiple_of(jj * R, R)
            q0 = jj * 2 * M
            xn = _bf(xn_ref[pl.ds(pl.multiple_of(jj * SEG, SEG), SEG), :]).astype(F32)
            jn = jnp.minimum(jj + 1, S // R - 1)
            tparts, tnext, gate = list(tcar), [], []

            def cur(c):
                return lambda: tparts.append(gcol(jj, c))

            def nxt(c):
                return lambda: tnext.append(gcol(jn, c))

            def gout():
                u = _dot(jnp.concatenate(tparts, axis=1), wout_ref[...])
                gate.append(u * jax.nn.sigmoid(u))

            stash_kv, stash_o = {}, {}

            hA = jnp.concatenate([mem, xn[:SEG + M]], axis=0).astype(BF16)

            def projA(p):
                q = _dot(hA[:SEG], wpair((0,), p))
                kv = _dot(hA, wpair((1, 2), p))
                stash_kv[p] = kv[L:]
                kv = kv[:L]
                q = jnp.concatenate([q, qpre_rows(p, q0)], axis=0)
                return stack(q, 0), stack(kv, 0), stack(kv, 2)

            def preA(p, o):
                stash_o[p] = o[SEG:]
                return o[:SEG]

            accA = run_step(projA, preA, [cur(2), cur(3), cur(4), cur(5)])

            hB = jnp.concatenate([accA[:M], xn[SEG + M:]], axis=0).astype(BF16)

            def projB(p):
                r = _dot(hB, wpair((0, 1, 2), p))
                st = jnp.concatenate([qpre_rows(p, q0 + M), stash_kv[p]], axis=1)
                r = jnp.concatenate([r[:M], st, r[M:]], axis=0)
                return stack(r, 0), stack(r, 2), stack(r, 4)

            def preB(p, o):
                return jnp.concatenate([o, stash_o[p]], axis=0)

            accB = run_step(projB, preB, [cur(6), nxt(0), gout, nxt(1)])

            s_out = jnp.concatenate([accA[M:], accB[L:], accB[M:L]], axis=0)
            xr = x_ref[pl.ds(r0, R), :].astype(F32)
            o_ref[pl.ds(r0, R), :] = (xr + s_out * gate[0]).astype(o_ref.dtype)
            return accB[:M], tuple(tnext)

        for uu in range(UNR):
            carry = pair_step(it * UNR + uu, *carry)
        out_copy(it).start()
        return carry

    nit = GRID or NIT
    jax.lax.fori_loop(0, nit, main, (mem0_ref[0].astype(F32), t_init))
    for i in range(nit):
        out_copy(i).wait()
    for i in range(nit + 1, NIT):
        wsp_copy(i).wait()


@functools.partial(jax.jit, static_argnames=("SEG",))
def _run(A_x, A_mem0, A_Wq, A_Wk, A_Wv, A_Wo, B_w_in, B_w_sp, B_b_sp, B_w_out, *, SEG):
    B, S, D = A_x.shape
    H, Dh = A_Wq.shape[1], A_Wq.shape[2]
    M = A_mem0.shape[1]
    FH = B_w_in.shape[1] // 2
    assert (B, S, D, H, Dh, M, SEG, FH) == (1, 2048, 640, 32, 128, 8, 32, 864)
    wq, wk, wv = (w.reshape(D * H, Dh) for w in (A_Wq, A_Wk, A_Wv))
    wo = A_Wo.reshape(H * Dh, D)
    b = B_b_sp.reshape(S // 128, 128)
    win_t = B_w_in.T
    NS = S // SEG * M
    RS = D // 2 + RPAD
    NIT = S // (2 * SEG * UNR)
    anyspec = pl.BlockSpec(memory_space=pl.ANY)
    return pl.pallas_call(
        functools.partial(_kernel, S=S, D=D, H=H, Dh=Dh, M=M, SEG=SEG, FH=FH),
        in_specs=[anyspec] * 10,
        out_specs=anyspec,
        out_shape=jax.ShapeDtypeStruct(A_x.shape, A_x.dtype),
        scratch_shapes=[
            pltpu.VMEM((S, D), BF16),
            pltpu.VMEM((S // 2, D), U32),
            pltpu.VMEM((NS, D), BF16),
            pltpu.VMEM((H * RS + -(-FH // 128) * (S // 2), Dh), U32),
            pltpu.VMEM((2 * H * RS + H * NS, Dh), U32),
            pltpu.VMEM((S // 2, FH), U32),
            pltpu.VMEM(A_mem0.shape, BF16),
            pltpu.VMEM((3, D * H, Dh), BF16),
            pltpu.VMEM(wo.shape, BF16),
            pltpu.VMEM(win_t.shape, BF16),
            pltpu.VMEM(B_w_sp.shape, BF16),
            pltpu.VMEM(B_w_out.shape, BF16),
            pltpu.VMEM(b.shape, BF16),
            pltpu.VMEM((S, 128), F32),
            pltpu.VMEM((S, D), BF16),
            pltpu.SemaphoreType.DMA((12 + S // (SB * ZU) + 2 * NIT,)),
        ],
        compiler_params=pltpu.CompilerParams(vmem_limit_bytes=110 * 1024 * 1024),
        interpret=INTERPRET,
    )(A_x, A_mem0, wq, wk, wv, wo, win_t, B_w_sp, b, B_w_out)


def pallas_recurrent_scan__memory_aug_recurrent_mem_tr__mixer_gmlp__prompt_kernel(A_x, A_mem0, A_Wq, A_Wk, A_Wv, A_Wo, A_seg_len, B_x, B_w_in, B_w_sp, B_b_sp, B_w_out):
    seg = A_seg_len if isinstance(A_seg_len, int) else 32
    return _run(A_x, A_mem0, A_Wq, A_Wk, A_Wv, A_Wo, B_w_in, B_w_sp, B_b_sp, B_w_out, SEG=seg)
```

```python
import functools
import math

import jax
import jax.numpy as jnp
import jax.experimental.pallas as pl
import jax.experimental.pallas.tpu as pltpu

F32 = jnp.float32
BF16 = jnp.bfloat16
U32 = jnp.uint32

RPAD = 4
UNR = 2
SB = 128
ZU = 4
PG = 8
NCH = 4
NCAR = 2
ZORD0 = (0, 3, 1, 2)
ZORD = [(1, 0), (1, 1), (1, 2), (2, 3), (2, 0), (2, 1), (2, 2), (1, 3)]
XA = 3


def _ln(x, eps=1e-5):
    m = jnp.mean(x, axis=-1, keepdims=True)
    xc = x - m
    v = jnp.mean(xc * xc, axis=-1, keepdims=True)
    return xc * jax.lax.rsqrt(v + eps)


def _dot(a, b):
    return jnp.dot(a, b, preferred_element_type=F32)


def _dot_t(a, b):
    return jax.lax.dot_general(a, b, (((1,), (1,)), ((), ())), preferred_element_type=F32)


def _bf(u):
    return pltpu.bitcast(u, BF16)


def _pk(x):
    return pltpu.bitcast(x, U32)


def _gelu(x):
    c0 = math.sqrt(2.0 / math.pi)
    u = x * (x * x * (c0 * 0.044715) + c0)
    h = 0.5 * x
    return h * jnp.tanh(u) + h


def _mult(i, k):
    return i if isinstance(i, int) else pl.multiple_of(i, k)


def _kernel(x_hbm, mem0_hbm, wq_hbm, wk_hbm, wv_hbm, wo_hbm, win_hbm, wsp_hbm, b_hbm, wout_hbm,
            o_hbm,
            x_ref, xn_ref, xs_ref, wq_ref, wkv_ref, z2_ref, mem0_ref, wraw_ref, wo_ref, win_ref,
            wsp_ref, wout_ref, b_ref, btab_ref, o_ref, tc_ref, sems,
            *, S, D, H, Dh, M, SEG, FH):
    L = M + SEG
    R = 2 * SEG
    RU = R * UNR
    NIT = S // RU
    NP = H // 2
    HG = NP // 2
    DH2 = D // 2
    RS = DH2 + RPAD
    QL = SEG - M
    NS = S // R * 2 * M
    NX = SB // R * 2 * M
    edges = list(range(0, FH, 128)) + [FH]
    NT = len(edges) - 1
    NB = S // SB
    NZ = NB // ZU
    ZOFF = H * RS
    QOFF = 2 * H * RS
    WQP = D * H // NZ

    sem_ids = iter(range(sems.shape[0]))

    def sem_block(n):
        return [next(sem_ids) for _ in range(n)][0]

    def rows_copy(src, dst, lo, n, sem):
        return pltpu.make_async_copy(src.at[pl.ds(lo, n), :], dst.at[pl.ds(lo, n), :], sems.at[sem])

    def full_copy(src, dst):
        return pltpu.make_async_copy(src, dst, sems.at[sem_block(1)])

    x2 = x_hbm.at[0]
    xa_copy = rows_copy(x2, x_ref, 0, XA * SB, sem_block(1))
    xb_copy = rows_copy(x2, x_ref, XA * SB, (ZU + 1 - XA) * SB, sem_block(1))
    xc_copy = rows_copy(x2, x_ref, (ZU + 1) * SB, ZU * SB, sem_block(1))
    xd_copy = rows_copy(x2, x_ref, (2 * ZU + 1) * SB, S - (2 * ZU + 1) * SB, sem_block(1))
    win1_copy = rows_copy(win_hbm, win_ref, 0, FH, sem_block(1))
    win2_copy = rows_copy(win_hbm, win_ref, FH, FH, sem_block(1))
    wk_copy = full_copy(wk_hbm, wraw_ref.at[1])
    wv_copy = full_copy(wv_hbm, wraw_ref.at[2])
    wo_copy = full_copy(wo_hbm, wo_ref)
    wout_copy = full_copy(wout_hbm, wout_ref)
    mem0_copy = full_copy(mem0_hbm, mem0_ref)
    b_copy = full_copy(b_hbm, b_ref)
    wspa_copy = rows_copy(wsp_hbm, wsp_ref, 0, RU + R, sem_block(1))
    wspb_copy = rows_copy(wsp_hbm, wsp_ref, RU + R, S - RU - R, sem_block(1))
    wq_sem, out_sem = sem_block(NZ), sem_block(1)

    def wq_copy(c):
        return rows_copy(wq_hbm, wraw_ref.at[0], c * WQP, WQP, wq_sem + c)

    def out_copy(i):
        return rows_copy(o_ref, o_hbm.at[0], i * RU, RU, out_sem)

    for c in ([b_copy, xa_copy, win1_copy, mem0_copy, win2_copy, xb_copy, xc_copy, wq_copy(0), wq_copy(1), xd_copy]
              + [wq_copy(c) for c in range(2, NZ)] + [wk_copy, wv_copy, wo_copy, wout_copy, wspa_copy, wspb_copy]):
        c.start()

    def wdst(w):
        return (wq_ref, 0) if isinstance(w, int) and w == 0 else (wkv_ref, (w - 1) * H)

    def wpair(ws, p):
        parts = []
        for w in ws:
            ref, h0 = wdst(w)
            for par in range(2):
                parts.append(_bf(ref[pl.ds((h0 + par * NP + p) * RS, DH2), :]))
        return jnp.concatenate(parts, axis=1)

    def relayout(w, grp, j0, nj):
        src = wraw_ref.at[w, pl.ds(pl.multiple_of((j0 * H + grp * HG) * 2, HG * 2), (nj * H - HG) * 2), :]
        dst, h0 = wdst(w)
        base = (h0 + grp * HG) * RS + j0
        for u in range(nj):
            a = _pk(src[u * H * 2:(u * H + HG) * 2, :])
            b = _pk(src[(u * H + NP) * 2:(u * H + NP + HG) * 2, :])
            dst[pl.ds(base + u, HG, stride=RS), :] = (a & jnp.uint32(0xFFFF)) | (b << 16)
            dst[pl.ds(base + NP * RS + u, HG, stride=RS), :] = (a >> 16) | (b & jnp.uint32(0xFFFF0000))

    class Blk:
        def __init__(self, i0, n):
            v = lambda ref, k: ref.at[pl.ds(_mult(i0 * k, k), n * k), :]
            self.x, self.xn, self.xs, self.z2 = v(x_ref, SB), v(xn_ref, SB // 2), v(xs_ref, NX // 2), v(z2_ref, SB // 2)
            self.i0 = i0

        def ln(self, s):
            xn = _ln(self.x[s * SB:(s + 1) * SB, :].astype(F32))
            xb = xn.astype(BF16)
            self.xn[s * SB // 2:(s + 1) * SB // 2, :] = _pk(xb)
            sel = jnp.concatenate([xn[k * R + QL:k * R + QL + 2 * M] for k in range(SB // R)], axis=0)
            self.xs[s * NX // 2:(s + 1) * NX // 2, :] = _pk(sel.astype(BF16))
            return xb

        def z2_rows(self, s, xb):
            z2 = _ln(_gelu(_dot_t(xb, win_ref[FH:, :])))
            self.z2[s * SB // 2:(s + 1) * SB // 2, :] = _pk(z2.astype(BF16))

        def z1_rows(self, s, xb, extra=None):
            z1 = _dot_t(xb, win_ref[:FH, :])
            r = (self.i0 + s) * (SB // 2)
            for c in range(NT):
                wq_ref[pl.ds(_mult(ZOFF + c * (S // 2) + r, 8), SB // 2), :edges[c + 1] - edges[c]] = (
                    _pk(z1[:, edges[c]:edges[c + 1]].astype(BF16)))
                if extra is not None:
                    extra(c)

    blk0 = Blk(0, ZU + 1)
    xa_copy.wait()
    xbs = [blk0.ln(i) for i in range(XA)]
    b_copy.wait()
    bt = jnp.transpose(jnp.concatenate([b_ref[...].astype(F32)] * (128 * 128 // S), axis=0))
    for i in range(S // 128):
        btab_ref[i * 128:(i + 1) * 128, :] = jnp.broadcast_to(bt[:, i:i + 1], (128, 128))
    win1_copy.wait()
    for i in range(min(XA, ZU - 1)):
        blk0.z1_rows(i, xbs[i])
    win2_copy.wait()
    xb_copy.wait()
    for i in range(XA, ZU + 1):
        xbs.append(blk0.ln(i))
    for i in ZORD0:
        blk0.z2_rows(i, xbs[i])
    for i in range(min(XA, ZU - 1), ZU):
        blk0.z1_rows(i, xbs[i])
    xc_copy.wait()
    wq_copy(0).wait()
    CJ = -(-DH2 // ((NZ - 1) * ZU * NT))

    def zgroup(c, carry):
        wq_copy(c).wait()

        @pl.when(c == 2)
        def _():
            xd_copy.wait()

        blk = Blk(c * ZU, ZU)
        xbs = [_bf(blk.xn[:SB // 2, :])]
        for s in range(1, ZU):
            xbs.append(blk.ln(s))
        Blk(jnp.minimum((c + 1) * ZU, NB - 1), 1).ln(0)
        n1 = 0
        for kind, s in ZORD:
            if kind == 2:
                blk.z2_rows(s, xbs[s])
            else:
                def extra(t):
                    j0 = jnp.minimum((((c - 1) * ZU + n1) * NT + t) * CJ, DH2 - CJ)
                    relayout(0, 0, j0, CJ)
                    relayout(0, 1, j0, CJ)
                blk.z1_rows(s, xbs[s], extra)
                n1 += 1
        return carry
    jax.lax.fori_loop(1, NZ, zgroup, 0)

    wk_copy.wait()
    wv_copy.wait()
    UPP = NP // 4
    NJ = DH2 // UPP

    def qpre(i, carry):
        xs = _bf(xs_ref[...])
        nr = NS // NCH
        nj = NJ // (2 * NCH)
        for k in range(PG):
            p = i * PG + k
            unit = p // UPP
            q = _dot(xs, wpair((0,), p))
            for par in range(2):
                for c in range(NCH):
                    wkv_ref[pl.ds(pl.multiple_of(QOFF + (2 * p + par) * NS + c * nr, 8), nr), :] = _pk(
                        q[c * nr:(c + 1) * nr, par * Dh:(par + 1) * Dh])
                    relayout(1 + unit // 2, unit % 2, (p % UPP) * NJ + (par * NCH + c) * nj, nj)
        return carry
    jax.lax.fori_loop(0, NP // PG, qpre, 0)

    def qpre_rows(p, r):
        return jnp.concatenate(
            [pltpu.bitcast(wkv_ref[pl.ds(pl.multiple_of(QOFF + (2 * p + par) * NS + r, 8), M), :], F32)
             for par in range(2)], axis=1)

    def gcol(jj, c):
        r0 = _mult(jj * R, R)
        w = edges[c + 1] - edges[c]
        g = _dot(wsp_ref[pl.ds(r0, R), :], _bf(z2_ref[:, edges[c]:edges[c + 1]])) + btab_ref[pl.ds(r0, R), :w]
        z1 = _bf(wq_ref[pl.ds(_mult(ZOFF + c * (S // 2) + jj * SEG, 8), SEG), :w]).astype(F32)
        return (_gelu(z1) * g).astype(BF16)

    wo_copy.wait()
    wout_copy.wait()
    mem0_copy.wait()
    wspa_copy.wait()
    for c in range(NCAR):
        tc_ref[:, c * 128:(c + 1) * 128] = _pk(gcol(0, c))

    scale = Dh ** -0.5
    c_exp = scale * math.log2(math.e)

    def main(it, mem):
        @pl.when(it == 1)
        def _():
            wspb_copy.wait()

        row = jax.lax.broadcasted_iota(jnp.int32, (2 * L, 2 * L), 0)
        col = jax.lax.broadcasted_iota(jnp.int32, (2 * L, 2 * L), 1)
        rhi = row >= L
        chi = col >= L
        rl = jnp.where(rhi, row - L, row)
        cl = jnp.where(chi, col - L, col)
        same = rhi == chi
        valid = same & ((rl < M) | (rl >= cl))
        fill = jnp.where(same, -1e9 / scale, -jnp.inf).astype(F32)

        def stack(a, i):
            return jnp.concatenate([a[:, i * Dh:(i + 1) * Dh], a[:, (i + 1) * Dh:(i + 2) * Dh]], axis=0).astype(BF16)

        def scores(q2, k2):
            s = jnp.where(valid, _dot_t(q2, k2), fill)
            m = jnp.max(s, axis=-1, keepdims=True)
            e = jnp.exp2((s - m) * c_exp)
            l = jnp.sum(e, axis=-1, keepdims=True)
            return e.astype(BF16), 1.0 / l

        def pv(e, inv_l, v2):
            o2 = _dot(e, v2) * inv_l
            return jnp.concatenate([o2[:L], o2[L:]], axis=1)

        def run_step(proj, pre_o, fillers):
            qkv, sm, oo = {}, {}, {}
            acc = None
            for t in range(NP + 3):
                if t < NP:
                    qkv[t] = proj(t)
                else:
                    fillers[t - NP]()
                p = t - 3
                if 0 <= p < NP:
                    tt = _dot(oo[p], wo_ref[p * 2 * Dh:(p + 1) * 2 * Dh, :])
                    acc = tt if acc is None else acc + tt
                p = t - 1
                if 0 <= p < NP:
                    sm[p] = scores(qkv[p][0], qkv[p][1])
                p = t - 2
                if 0 <= p < NP:
                    oo[p] = pre_o(p, pv(sm[p][0], sm[p][1], qkv[p][2])).astype(BF16)
            fillers[3]()
            return acc

        def pair_step(jj, mem, tcar):
            r0 = pl.multiple_of(jj * R, R)
            q0 = jj * 2 * M
            xn = _bf(xn_ref[pl.ds(pl.multiple_of(jj * SEG, SEG), SEG), :]).astype(F32)
            jn = jnp.minimum(jj + 1, S // R - 1)
            tparts, tnext, gate = list(tcar), [], []

            def cur(c):
                return lambda: tparts.append(gcol(jj, c))

            def nxt(c):
                return lambda: tnext.append(gcol(jn, c))

            def gout():
                u = _dot(jnp.concatenate(tparts, axis=1), wout_ref[...])
                gate.append(u * jax.nn.sigmoid(u))

            stash_kv, stash_o = {}, {}

            hA = jnp.concatenate([mem, xn[:SEG + M]], axis=0).astype(BF16)

            def projA(p):
                q = _dot(hA[:SEG], wpair((0,), p))
                kv = _dot(hA, wpair((1, 2), p))
                stash_kv[p] = kv[L:]
                kv = kv[:L]
                q = jnp.concatenate([q, qpre_rows(p, q0)], axis=0)
                return stack(q, 0), stack(kv, 0), stack(kv, 2)

            def preA(p, o):
                stash_o[p] = o[SEG:]
                return o[:SEG]

            accA = run_step(projA, preA, [cur(2), cur(3), cur(4), cur(5)])

            hB = jnp.concatenate([accA[:M], xn[SEG + M:]], axis=0).astype(BF16)

            def projB(p):
                r = _dot(hB, wpair((0, 1, 2), p))
                st = jnp.concatenate([qpre_rows(p, q0 + M), stash_kv[p]], axis=1)
                r = jnp.concatenate([r[:M], st, r[M:]], axis=0)
                return stack(r, 0), stack(r, 2), stack(r, 4)

            def preB(p, o):
                return jnp.concatenate([o, stash_o[p]], axis=0)

            accB = run_step(projB, preB, [cur(6), nxt(0), gout, nxt(1)])

            s_out = jnp.concatenate([accA[M:], accB[L:], accB[M:L]], axis=0)
            xr = x_ref[pl.ds(r0, R), :].astype(F32)
            o_ref[pl.ds(r0, R), :] = (xr + s_out * gate[0]).astype(o_ref.dtype)
            return accB[:M], tuple(tnext)

        tcar = tuple(_bf(tc_ref[:, c * 128:(c + 1) * 128]) for c in range(NCAR))
        for uu in range(UNR):
            mem, tcar = pair_step(it * UNR + uu, mem, tcar)
        out_copy(it).start()
        for c in range(NCAR):
            tc_ref[:, c * 128:(c + 1) * 128] = _pk(tcar[c])
        return mem

    jax.lax.fori_loop(0, NIT, main, mem0_ref[0].astype(F32))
    for i in range(NIT):
        out_copy(i).wait()


@functools.partial(jax.jit, static_argnames=("SEG",))
def _run(A_x, A_mem0, A_Wq, A_Wk, A_Wv, A_Wo, B_w_in, B_w_sp, B_b_sp, B_w_out, *, SEG):
    B, S, D = A_x.shape
    H, Dh = A_Wq.shape[1], A_Wq.shape[2]
    M = A_mem0.shape[1]
    FH = B_w_in.shape[1] // 2
    assert (B, S, D, H, Dh, M, SEG, FH) == (1, 2048, 640, 32, 128, 8, 32, 864)
    wq, wk, wv = (w.reshape(D * H, Dh) for w in (A_Wq, A_Wk, A_Wv))
    wo = A_Wo.reshape(H * Dh, D)
    b = B_b_sp.reshape(S // 128, 128)
    win_t = B_w_in.T
    NS = S // SEG * M
    RS = D // 2 + RPAD
    NIT = S // (2 * SEG * UNR)
    anyspec = pl.BlockSpec(memory_space=pl.ANY)
    return pl.pallas_call(
        functools.partial(_kernel, S=S, D=D, H=H, Dh=Dh, M=M, SEG=SEG, FH=FH),
        in_specs=[anyspec] * 10,
        out_specs=anyspec,
        out_shape=jax.ShapeDtypeStruct(A_x.shape, A_x.dtype),
        scratch_shapes=[
            pltpu.VMEM((S, D), BF16),
            pltpu.VMEM((S // 2, D), U32),
            pltpu.VMEM((NS // 2, D), U32),
            pltpu.VMEM((H * RS + -(-FH // 128) * (S // 2), Dh), U32),
            pltpu.VMEM((2 * H * RS + H * NS, Dh), U32),
            pltpu.VMEM((S // 2, FH), U32),
            pltpu.VMEM(A_mem0.shape, BF16),
            pltpu.VMEM((3, D * H, Dh), BF16),
            pltpu.VMEM(wo.shape, BF16),
            pltpu.VMEM(win_t.shape, BF16),
            pltpu.VMEM(B_w_sp.shape, BF16),
            pltpu.VMEM(B_w_out.shape, BF16),
            pltpu.VMEM(b.shape, BF16),
            pltpu.VMEM((S, 128), F32),
            pltpu.VMEM((S, D), BF16),
            pltpu.VMEM((SEG, NCAR * 128), U32),
            pltpu.SemaphoreType.DMA((15 + S // (SB * ZU),)),
        ],
        compiler_params=pltpu.CompilerParams(vmem_limit_bytes=110 * 1024 * 1024),
    )(A_x, A_mem0, wq, wk, wv, wo, win_t, B_w_sp, b, B_w_out)


def pallas_recurrent_scan__memory_aug_recurrent_mem_tr__mixer_gmlp__prompt_kernel(
        A_x, A_mem0, A_Wq, A_Wk, A_Wv, A_Wo, A_seg_len, B_x, B_w_in, B_w_sp, B_b_sp, B_w_out):
    seg = A_seg_len if isinstance(A_seg_len, int) else 32
    return _run(A_x, A_mem0, A_Wq, A_Wk, A_Wv, A_Wo, B_w_in, B_w_sp, B_b_sp, B_w_out, SEG=seg)
```

```python
import functools
import math

import jax
import jax.numpy as jnp
import jax.experimental.pallas as pl
import jax.experimental.pallas.tpu as pltpu

F32 = jnp.float32
BF16 = jnp.bfloat16
U32 = jnp.uint32

RPAD = 4
UNR = 2
SB = 128
ZU = 4
PG = 8
NCH = 4
NCAR = 2
W0 = 3
ZORD0 = (0, 3, 1, 2)
ZORD = [(1, 0), (1, 1), (1, 2), (2, 3), (2, 0), (2, 1), (2, 2), (1, 3)]
XA = 3


def _ln(x, eps=1e-5):
    m = jnp.mean(x, axis=-1, keepdims=True)
    xc = x - m
    v = jnp.mean(xc * xc, axis=-1, keepdims=True)
    return xc * jax.lax.rsqrt(v + eps)


def _dot(a, b):
    return jnp.dot(a, b, preferred_element_type=F32)


def _dot_t(a, b):
    return jax.lax.dot_general(a, b, (((1,), (1,)), ((), ())), preferred_element_type=F32)


def _bf(u):
    return pltpu.bitcast(u, BF16)


def _pk(x):
    return pltpu.bitcast(x, U32)


def _gelu(x):
    c0 = math.sqrt(2.0 / math.pi)
    u = x * (x * x * (c0 * 0.044715) + c0)
    h = 0.5 * x
    return h * jnp.tanh(u) + h


def _mult(i, k):
    return i if isinstance(i, int) else pl.multiple_of(i, k)


def _kernel(x_hbm, mem0_hbm, wq_hbm, wk_hbm, wv_hbm, wo_hbm, win_hbm, wsp_hbm, b_hbm, wout_hbm,
            o_hbm,
            x_ref, xn_ref, xs_ref, wq_ref, wkv_ref, z2_ref, mem0_ref, wraw_ref, wo_ref, win_ref,
            wsp_ref, wout_ref, b_ref, btab_ref, o_ref, tc_ref, sems,
            *, S, D, H, Dh, M, SEG, FH):
    L = M + SEG
    R = 2 * SEG
    RU = R * UNR
    NIT = S // RU
    NP = H // 2
    HG = NP // 2
    DH2 = D // 2
    RS = DH2 + RPAD
    QL = SEG - M
    NS = S // R * 2 * M
    NX = SB // R * 2 * M
    edges = list(range(0, FH, 128)) + [FH]
    NT = len(edges) - 1
    NB = S // SB
    NZ = NB // ZU
    ZOFF = H * RS
    QOFF = 2 * H * RS
    CJ = -(-DH2 // ((NZ - 1) * ZU * NT))
    WQP = CJ * ZU * NT * 2 * H

    sem_ids = iter(range(sems.shape[0]))

    def sem_block(n):
        return [next(sem_ids) for _ in range(n)][0]

    def rows_copy(src, dst, lo, n, sem):
        return pltpu.make_async_copy(src.at[pl.ds(lo, n), :], dst.at[pl.ds(lo, n), :], sems.at[sem])

    def full_copy(src, dst):
        return pltpu.make_async_copy(src, dst, sems.at[sem_block(1)])

    x2 = x_hbm.at[0]
    xa_copy = rows_copy(x2, x_ref, 0, XA * SB, sem_block(1))
    xb_copy = rows_copy(x2, x_ref, XA * SB, (ZU + 1 - XA) * SB, sem_block(1))
    xc_copy = rows_copy(x2, x_ref, (ZU + 1) * SB, ZU * SB, sem_block(1))
    xd_copy = rows_copy(x2, x_ref, (2 * ZU + 1) * SB, S - (2 * ZU + 1) * SB, sem_block(1))
    win0_copy = rows_copy(win_hbm, win_ref, 0, W0 * 128, sem_block(1))
    win1_copy = rows_copy(win_hbm, win_ref, W0 * 128, FH - W0 * 128, sem_block(1))
    win2_copy = rows_copy(win_hbm, win_ref, FH, FH, sem_block(1))
    wk_copy = full_copy(wk_hbm, wraw_ref.at[1])
    wv_copy = full_copy(wv_hbm, wraw_ref.at[2])
    wo_copy = full_copy(wo_hbm, wo_ref)
    wout_copy = full_copy(wout_hbm, wout_ref)
    mem0_copy = full_copy(mem0_hbm, mem0_ref)
    b_copy = full_copy(b_hbm, b_ref)
    wspa_copy = rows_copy(wsp_hbm, wsp_ref, 0, RU + R, sem_block(1))
    wspb_copy = rows_copy(wsp_hbm, wsp_ref, RU + R, S - RU - R, sem_block(1))
    wq_sem, out_sem = sem_block(NZ - 1), sem_block(1)

    def wq_copy(c):
        return rows_copy(wq_hbm, wraw_ref.at[0], c * WQP, min(WQP, D * H - c * WQP), wq_sem + c)

    def out_copy(i):
        return rows_copy(o_ref, o_hbm.at[0], i * RU, RU, out_sem)

    for c in ([b_copy, xa_copy, win0_copy, win1_copy, mem0_copy, win2_copy, xb_copy, xc_copy, wq_copy(0), xd_copy]
              + [wq_copy(c) for c in range(1, NZ - 1)] + [wk_copy, wv_copy, wo_copy, wout_copy, wspa_copy, wspb_copy]):
        c.start()

    def wdst(w):
        return (wq_ref, 0) if isinstance(w, int) and w == 0 else (wkv_ref, (w - 1) * H)

    def wpair(ws, p):
        parts = []
        for w in ws:
            ref, h0 = wdst(w)
            for par in range(2):
                parts.append(_bf(ref[pl.ds((h0 + par * NP + p) * RS, DH2), :]))
        return jnp.concatenate(parts, axis=1)

    def relayout(w, grp, j0, nj):
        src = wraw_ref.at[w, pl.ds(pl.multiple_of((j0 * H + grp * HG) * 2, HG * 2), (nj * H - HG) * 2), :]
        dst, h0 = wdst(w)
        base = (h0 + grp * HG) * RS + j0
        for u in range(nj):
            a = _pk(src[u * H * 2:(u * H + HG) * 2, :])
            b = _pk(src[(u * H + NP) * 2:(u * H + NP + HG) * 2, :])
            dst[pl.ds(base + u, HG, stride=RS), :] = (a & jnp.uint32(0xFFFF)) | (b << 16)
            dst[pl.ds(base + NP * RS + u, HG, stride=RS), :] = (a >> 16) | (b & jnp.uint32(0xFFFF0000))

    class Blk:
        def __init__(self, i0, n):
            v = lambda ref, k: ref.at[pl.ds(_mult(i0 * k, k), n * k), :]
            self.x, self.xn, self.xs, self.z2 = v(x_ref, SB), v(xn_ref, SB // 2), v(xs_ref, NX // 2), v(z2_ref, SB // 2)
            self.i0 = i0

        def ln(self, s):
            xn = _ln(self.x[s * SB:(s + 1) * SB, :].astype(F32))
            xb = xn.astype(BF16)
            self.xn[s * SB // 2:(s + 1) * SB // 2, :] = _pk(xb)
            sel = jnp.concatenate([xn[k * R + QL:k * R + QL + 2 * M] for k in range(SB // R)], axis=0)
            self.xs[s * NX // 2:(s + 1) * NX // 2, :] = _pk(sel.astype(BF16))
            return xb

        def z2_rows(self, s, xb):
            z2 = _ln(_gelu(_dot_t(xb, win_ref[FH:, :])))
            self.z2[s * SB // 2:(s + 1) * SB // 2, :] = _pk(z2.astype(BF16))

        def z1_rows(self, s, xb, extra=None, c0=0, c1=NT):
            z1 = _dot_t(xb, win_ref[edges[c0]:edges[c1], :])
            r = (self.i0 + s) * (SB // 2)
            for c in range(c0, c1):
                wq_ref[pl.ds(_mult(ZOFF + c * (S // 2) + r, 8), SB // 2), :edges[c + 1] - edges[c]] = (
                    _pk(z1[:, edges[c] - edges[c0]:edges[c + 1] - edges[c0]].astype(BF16)))
                if extra is not None:
                    extra(c)

    blk0 = Blk(0, ZU + 1)
    b_copy.wait()
    bt = jnp.transpose(jnp.concatenate([b_ref[...].astype(F32)] * (128 * 128 // S), axis=0))
    for i in range(S // 128):
        btab_ref[i * 128:(i + 1) * 128, :] = jnp.broadcast_to(bt[:, i:i + 1], (128, 128))
    xa_copy.wait()
    xbs = [blk0.ln(i) for i in range(XA)]
    win0_copy.wait()
    for i in range(XA):
        blk0.z1_rows(i, xbs[i], c1=W0)
    win1_copy.wait()
    for i in range(XA):
        blk0.z1_rows(i, xbs[i], c0=W0)
    win2_copy.wait()
    xb_copy.wait()
    for i in range(XA, ZU + 1):
        xbs.append(blk0.ln(i))
    for i in ZORD0:
        blk0.z2_rows(i, xbs[i])
    for i in range(min(XA, ZU - 1), ZU):
        blk0.z1_rows(i, xbs[i])
    xc_copy.wait()
    wq_copy(0).wait()

    def zgroup(c, carry):
        @pl.when(c == 2)
        def _():
            xd_copy.wait()
            wq_copy(1).wait()

        @pl.when(c == 3)
        def _():
            wq_copy(2).wait()

        blk = Blk(c * ZU, ZU)
        xbs = [_bf(blk.xn[:SB // 2, :])]
        for s in range(1, ZU):
            xbs.append(blk.ln(s))
        Blk(jnp.minimum((c + 1) * ZU, NB - 1), 1).ln(0)
        n1 = 0
        for kind, s in ZORD:
            if kind == 2:
                blk.z2_rows(s, xbs[s])
            else:
                def extra(t):
                    j0 = jnp.minimum((((c - 1) * ZU + n1) * NT + t) * CJ, DH2 - CJ)
                    relayout(0, 0, j0, CJ)
                    relayout(0, 1, j0, CJ)
                blk.z1_rows(s, xbs[s], extra)
                n1 += 1
        return carry
    jax.lax.fori_loop(1, NZ, zgroup, 0)

    wk_copy.wait()
    UPP = NP // 4
    NJ = DH2 // UPP

    def qpre(i, carry):
        @pl.when(i * PG == NP // 2)
        def _():
            wv_copy.wait()

        xs = _bf(xs_ref[...])
        nr = NS // NCH
        nj = NJ // (2 * NCH)
        for k in range(PG):
            p = i * PG + k
            unit = p // UPP
            q = _dot(xs, wpair((0,), p))
            for par in range(2):
                for c in range(NCH):
                    wkv_ref[pl.ds(pl.multiple_of(QOFF + (2 * p + par) * NS + c * nr, 8), nr), :] = _pk(
                        q[c * nr:(c + 1) * nr, par * Dh:(par + 1) * Dh])
                    relayout(1 + unit // 2, unit % 2, (p % UPP) * NJ + (par * NCH + c) * nj, nj)
        return carry
    jax.lax.fori_loop(0, NP // PG, qpre, 0)

    def qpre_rows(p, r):
        return jnp.concatenate(
            [pltpu.bitcast(wkv_ref[pl.ds(pl.multiple_of(QOFF + (2 * p + par) * NS + r, 8), M), :], F32)
             for par in range(2)], axis=1)

    def gcol(jj, c):
        r0 = _mult(jj * R, R)
        w = edges[c + 1] - edges[c]
        g = _dot(wsp_ref[pl.ds(r0, R), :], _bf(z2_ref[:, edges[c]:edges[c + 1]])) + btab_ref[pl.ds(r0, R), :w]
        z1 = _bf(wq_ref[pl.ds(_mult(ZOFF + c * (S // 2) + jj * SEG, 8), SEG), :w]).astype(F32)
        return (_gelu(z1) * g).astype(BF16)

    wo_copy.wait()
    wout_copy.wait()
    mem0_copy.wait()
    wspa_copy.wait()
    for c in range(NCAR):
        tc_ref[:, c * 128:(c + 1) * 128] = _pk(gcol(0, c))

    scale = Dh ** -0.5
    c_exp = scale * math.log2(math.e)

    def main(it, mem):
        @pl.when(it == 1)
        def _():
            wspb_copy.wait()

        row = jax.lax.broadcasted_iota(jnp.int32, (2 * L, 2 * L), 0)
        col = jax.lax.broadcasted_iota(jnp.int32, (2 * L, 2 * L), 1)
        rhi = row >= L
        chi = col >= L
        rl = jnp.where(rhi, row - L, row)
        cl = jnp.where(chi, col - L, col)
        same = rhi == chi
        valid = same & ((rl < M) | (rl >= cl))
        fill = jnp.where(same, -1e9 / scale, -jnp.inf).astype(F32)

        def stack(a, i):
            return jnp.concatenate([a[:, i * Dh:(i + 1) * Dh], a[:, (i + 1) * Dh:(i + 2) * Dh]], axis=0).astype(BF16)

        def scores(q2, k2):
            s = jnp.where(valid, _dot_t(q2, k2), fill)
            m = jnp.max(s, axis=-1, keepdims=True)
            e = jnp.exp2((s - m) * c_exp)
            l = jnp.sum(e, axis=-1, keepdims=True)
            return e.astype(BF16), 1.0 / l

        def pv(e, inv_l, v2):
            o2 = _dot(e, v2) * inv_l
            return jnp.concatenate([o2[:L], o2[L:]], axis=1)

        def run_step(proj, pre_o, fillers):
            qkv, sm, oo = {}, {}, {}
            acc = None
            for t in range(NP + 3):
                if t < NP:
                    qkv[t] = proj(t)
                else:
                    fillers[t - NP]()
                p = t - 3
                if 0 <= p < NP:
                    tt = _dot(oo[p], wo_ref[p * 2 * Dh:(p + 1) * 2 * Dh, :])
                    acc = tt if acc is None else acc + tt
                p = t - 1
                if 0 <= p < NP:
                    sm[p] = scores(qkv[p][0], qkv[p][1])
                p = t - 2
                if 0 <= p < NP:
                    oo[p] = pre_o(p, pv(sm[p][0], sm[p][1], qkv[p][2])).astype(BF16)
            fillers[3]()
            return acc

        def pair_step(jj, mem, tcar):
            r0 = pl.multiple_of(jj * R, R)
            q0 = jj * 2 * M
            xn = _bf(xn_ref[pl.ds(pl.multiple_of(jj * SEG, SEG), SEG), :]).astype(F32)
            jn = jnp.minimum(jj + 1, S // R - 1)
            tparts, tnext, gate = list(tcar), [], []

            def cur(c):
                return lambda: tparts.append(gcol(jj, c))

            def nxt(c):
                return lambda: tnext.append(gcol(jn, c))

            def gout():
                u = _dot(jnp.concatenate(tparts, axis=1), wout_ref[...])
                gate.append(u * jax.nn.sigmoid(u))

            stash_kv, stash_o = {}, {}

            hA = jnp.concatenate([mem, xn[:SEG + M]], axis=0).astype(BF16)

            def projA(p):
                q = _dot(hA[:SEG], wpair((0,), p))
                kv = _dot(hA, wpair((1, 2), p))
                stash_kv[p] = kv[L:]
                kv = kv[:L]
                q = jnp.concatenate([q, qpre_rows(p, q0)], axis=0)
                return stack(q, 0), stack(kv, 0), stack(kv, 2)

            def preA(p, o):
                stash_o[p] = o[SEG:]
                return o[:SEG]

            accA = run_step(projA, preA, [cur(2), cur(3), cur(4), cur(5)])

            hB = jnp.concatenate([accA[:M], xn[SEG + M:]], axis=0).astype(BF16)

            def projB(p):
                r = _dot(hB, wpair((0, 1, 2), p))
                st = jnp.concatenate([qpre_rows(p, q0 + M), stash_kv[p]], axis=1)
                r = jnp.concatenate([r[:M], st, r[M:]], axis=0)
                return stack(r, 0), stack(r, 2), stack(r, 4)

            def preB(p, o):
                return jnp.concatenate([o, stash_o[p]], axis=0)

            accB = run_step(projB, preB, [cur(6), nxt(0), gout, nxt(1)])

            s_out = jnp.concatenate([accA[M:], accB[L:], accB[M:L]], axis=0)
            xr = x_ref[pl.ds(r0, R), :].astype(F32)
            o_ref[pl.ds(r0, R), :] = (xr + s_out * gate[0]).astype(o_ref.dtype)
            return accB[:M], tuple(tnext)

        tcar = tuple(_bf(tc_ref[:, c * 128:(c + 1) * 128]) for c in range(NCAR))
        for uu in range(UNR):
            mem, tcar = pair_step(it * UNR + uu, mem, tcar)
        out_copy(it).start()
        for c in range(NCAR):
            tc_ref[:, c * 128:(c + 1) * 128] = _pk(tcar[c])
        return mem

    jax.lax.fori_loop(0, NIT, main, mem0_ref[0].astype(F32))
    for i in range(NIT):
        out_copy(i).wait()


@functools.partial(jax.jit, static_argnames=("SEG",))
def _run(A_x, A_mem0, A_Wq, A_Wk, A_Wv, A_Wo, B_w_in, B_w_sp, B_b_sp, B_w_out, *, SEG):
    B, S, D = A_x.shape
    H, Dh = A_Wq.shape[1], A_Wq.shape[2]
    M = A_mem0.shape[1]
    FH = B_w_in.shape[1] // 2
    assert (B, S, D, H, Dh, M, SEG, FH) == (1, 2048, 640, 32, 128, 8, 32, 864)
    wq, wk, wv = (w.reshape(D * H, Dh) for w in (A_Wq, A_Wk, A_Wv))
    wo = A_Wo.reshape(H * Dh, D)
    b = B_b_sp.reshape(S // 128, 128)
    win_t = B_w_in.T
    NS = S // SEG * M
    RS = D // 2 + RPAD
    anyspec = pl.BlockSpec(memory_space=pl.ANY)
    return pl.pallas_call(
        functools.partial(_kernel, S=S, D=D, H=H, Dh=Dh, M=M, SEG=SEG, FH=FH),
        in_specs=[anyspec] * 10,
        out_specs=anyspec,
        out_shape=jax.ShapeDtypeStruct(A_x.shape, A_x.dtype),
        scratch_shapes=[
            pltpu.VMEM((S, D), BF16),
            pltpu.VMEM((S // 2, D), U32),
            pltpu.VMEM((NS // 2, D), U32),
            pltpu.VMEM((H * RS + -(-FH // 128) * (S // 2), Dh), U32),
            pltpu.VMEM((2 * H * RS + H * NS, Dh), U32),
            pltpu.VMEM((S // 2, FH), U32),
            pltpu.VMEM(A_mem0.shape, BF16),
            pltpu.VMEM((3, D * H, Dh), BF16),
            pltpu.VMEM(wo.shape, BF16),
            pltpu.VMEM(win_t.shape, BF16),
            pltpu.VMEM(B_w_sp.shape, BF16),
            pltpu.VMEM(B_w_out.shape, BF16),
            pltpu.VMEM(b.shape, BF16),
            pltpu.VMEM((S, 128), F32),
            pltpu.VMEM((S, D), BF16),
            pltpu.VMEM((SEG, NCAR * 128), U32),
            pltpu.SemaphoreType.DMA((15 + S // (SB * ZU),)),
        ],
        compiler_params=pltpu.CompilerParams(vmem_limit_bytes=110 * 1024 * 1024),
    )(A_x, A_mem0, wq, wk, wv, wo, win_t, B_w_sp, b, B_w_out)


def pallas_recurrent_scan__memory_aug_recurrent_mem_tr__mixer_gmlp__prompt_kernel(
        A_x, A_mem0, A_Wq, A_Wk, A_Wv, A_Wo, A_seg_len, B_x, B_w_in, B_w_sp, B_b_sp, B_w_out):
    seg = A_seg_len if isinstance(A_seg_len, int) else 32
    return _run(A_x, A_mem0, A_Wq, A_Wk, A_Wv, A_Wo, B_w_in, B_w_sp, B_b_sp, B_w_out, SEG=seg)
```

```python
import functools
import math

import jax
import jax.numpy as jnp
import jax.experimental.pallas as pl
import jax.experimental.pallas.tpu as pltpu

F32 = jnp.float32
BF16 = jnp.bfloat16
U32 = jnp.uint32

RPAD = 4
UNR = 2
SB = 128
ZU = 4
PG = 8
NCH = 4
NCAR = 2
W1 = 3
GS = 256
W0 = 3
ZORD0 = (0, 3, 1, 2)
ZORD = [(1, 0), (1, 1), (1, 2), (2, 3), (2, 0), (2, 1), (2, 2), (1, 3)]
XA = 3


def _ln(x, eps=1e-5):
    m = jnp.mean(x, axis=-1, keepdims=True)
    xc = x - m
    v = jnp.mean(xc * xc, axis=-1, keepdims=True)
    return xc * jax.lax.rsqrt(v + eps)


def _dot(a, b):
    return jnp.dot(a, b, preferred_element_type=F32)


def _dot_t(a, b):
    return jax.lax.dot_general(a, b, (((1,), (1,)), ((), ())), preferred_element_type=F32)


def _bf(u):
    return pltpu.bitcast(u, BF16)


def _pk(x):
    return pltpu.bitcast(x, U32)


def _gelu(x):
    c0 = math.sqrt(2.0 / math.pi)
    u = x * (x * x * (c0 * 0.044715) + c0)
    h = 0.5 * x
    return h * jnp.tanh(u) + h


def _mult(i, k):
    return i if isinstance(i, int) else pl.multiple_of(i, k)


def _kernel(x_hbm, mem0_hbm, wq_hbm, wk_hbm, wv_hbm, wo_hbm, win_hbm, wsp_hbm, b_hbm, wout_hbm,
            o_hbm,
            x_ref, xn_ref, xs_ref, wq_ref, wkv_ref, z2_ref, z2t_ref, mem0_ref, wraw_ref, wo_ref, win_ref,
            wsp_ref, wout_ref, b_ref, btab_ref, o_ref, tc_ref, sems,
            *, S, D, H, Dh, M, SEG, FH):
    L = M + SEG
    R = 2 * SEG
    RU = R * UNR
    NIT = S // RU
    NP = H // 2
    HG = NP // 2
    DH2 = D // 2
    RS = DH2 + RPAD
    QL = SEG - M
    NS = S // R * 2 * M
    NX = SB // R * 2 * M
    NT = -(-FH // 128)
    FL = (NT - 1) * 128
    FP = FH - FL
    NB = S // SB
    NZ = NB // ZU
    ZOFF = H * RS
    QOFF = 2 * H * RS
    CJ = -(-DH2 // ((NZ - 1) * ZU * (NT - 1)))
    WQP = CJ * ZU * (NT - 1) * 2 * H

    sem_ids = iter(range(sems.shape[0]))

    def sem_block(n):
        return [next(sem_ids) for _ in range(n)][0]

    def rows_copy(src, dst, lo, n, sem):
        return pltpu.make_async_copy(src.at[pl.ds(lo, n), :], dst.at[pl.ds(lo, n), :], sems.at[sem])

    def full_copy(src, dst):
        return pltpu.make_async_copy(src, dst, sems.at[sem_block(1)])

    x2 = x_hbm.at[0]
    xa_copy = rows_copy(x2, x_ref, 0, XA * SB, sem_block(1))
    xb_copy = rows_copy(x2, x_ref, XA * SB, (ZU + 1 - XA) * SB, sem_block(1))
    xc_copy = rows_copy(x2, x_ref, (ZU + 1) * SB, ZU * SB, sem_block(1))
    xd_copy = rows_copy(x2, x_ref, (2 * ZU + 1) * SB, S - (2 * ZU + 1) * SB, sem_block(1))
    win0_copy = rows_copy(win_hbm, win_ref, 0, W0 * 128, sem_block(1))
    win1_copy = rows_copy(win_hbm, win_ref, W0 * 128, FH - W0 * 128, sem_block(1))
    win2_copy = rows_copy(win_hbm, win_ref, FH, FH, sem_block(1))
    wk_copy = full_copy(wk_hbm, wraw_ref.at[1])
    wv_copy = full_copy(wv_hbm, wraw_ref.at[2])
    wo_copy = full_copy(wo_hbm, wo_ref)
    wout_copy = full_copy(wout_hbm, wout_ref)
    mem0_copy = full_copy(mem0_hbm, mem0_ref)
    b_copy = full_copy(b_hbm, b_ref)
    wspa_copy = rows_copy(wsp_hbm, wsp_ref, 0, RU + R, sem_block(1))
    wspb_copy = rows_copy(wsp_hbm, wsp_ref, RU + R, S - RU - R, sem_block(1))
    wq_sem, out_sem = sem_block(NZ - 1), sem_block(1)

    def wq_copy(c):
        return rows_copy(wq_hbm, wraw_ref.at[0], c * WQP, min(WQP, D * H - c * WQP), wq_sem + c)

    def out_copy(i):
        return rows_copy(o_ref, o_hbm.at[0], i * RU, RU, out_sem)

    for c in ([b_copy, xa_copy, win0_copy, win1_copy, xb_copy, win2_copy, mem0_copy, xc_copy, wq_copy(0), xd_copy]
              + [wq_copy(c) for c in range(1, NZ - 1)] + [wk_copy, wv_copy, wo_copy, wout_copy, wspa_copy, wspb_copy]):
        c.start()

    def wdst(w):
        return (wq_ref, 0) if isinstance(w, int) and w == 0 else (wkv_ref, (w - 1) * H)

    def wpair(ws, p):
        parts = []
        for w in ws:
            ref, h0 = wdst(w)
            for par in range(2):
                parts.append(_bf(ref[pl.ds((h0 + par * NP + p) * RS, DH2), :]))
        return jnp.concatenate(parts, axis=1)

    def relayout(w, grp, j0, nj):
        src = wraw_ref.at[w, pl.ds(pl.multiple_of((j0 * H + grp * HG) * 2, HG * 2), (nj * H - HG) * 2), :]
        dst, h0 = wdst(w)
        base = (h0 + grp * HG) * RS + j0
        for u in range(nj):
            a = _pk(src[u * H * 2:(u * H + HG) * 2, :])
            b = _pk(src[(u * H + NP) * 2:(u * H + NP + HG) * 2, :])
            dst[pl.ds(base + u, HG, stride=RS), :] = (a & jnp.uint32(0xFFFF)) | (b << 16)
            dst[pl.ds(base + NP * RS + u, HG, stride=RS), :] = (a >> 16) | (b & jnp.uint32(0xFFFF0000))

    class Blk:
        def __init__(self, i0, n):
            v = lambda ref, k: ref.at[pl.ds(_mult(i0 * k, k), n * k), :]
            self.x, self.xn, self.xs, self.z2 = v(x_ref, SB), v(xn_ref, SB // 2), v(xs_ref, NX // 2), v(z2_ref, SB // 2)
            self.i0 = i0

        def ln(self, s):
            xn = _ln(self.x[s * SB:(s + 1) * SB, :].astype(F32))
            xb = xn.astype(BF16)
            self.xn[s * SB // 2:(s + 1) * SB // 2, :] = _pk(xb)
            sel = jnp.concatenate([xn[k * R + QL:k * R + QL + 2 * M] for k in range(SB // R)], axis=0)
            self.xs[s * NX // 2:(s + 1) * NX // 2, :] = _pk(sel.astype(BF16))
            return xb

        def z2_rows(self, s, xb):
            zt = _dot_t(jnp.concatenate([win_ref[FH + FL:, :], win_ref[FL:FH, :]], axis=0), xb)
            z1l = jnp.transpose(jnp.concatenate([zt[FP:], zt[:128 - FP]], axis=0))[:, :FP]
            wq_ref[pl.ds(_mult(ZOFF + (NT - 1) * (S // 2) + (self.i0 + s) * (SB // 2), 8), SB // 2), :FP] = (
                _pk(z1l.astype(BF16)))
            z2 = jnp.concatenate([_dot_t(xb, win_ref[FH:FH + FL, :]), jnp.transpose(zt[:128])[:, :FP]], axis=1)
            z2 = _ln(_gelu(z2))
            self.z2[s * SB // 2:(s + 1) * SB // 2, :] = _pk(z2[:, :FL].astype(BF16))
            z2t_ref[:, pl.ds(_mult((self.i0 + s) * SB, SB), SB)] = (
                _pk(jnp.transpose(z2[:, FH - 128:])[128 - FP:].astype(BF16)))

        def z1_rows(self, s, xb, extra=None, c0=0, c1=NT - 1):
            z1 = _dot_t(xb, win_ref[c0 * 128:c1 * 128, :])
            r = (self.i0 + s) * (SB // 2)
            for c in range(c0, c1):
                wq_ref[pl.ds(_mult(ZOFF + c * (S // 2) + r, 8), SB // 2), :] = (
                    _pk(z1[:, (c - c0) * 128:(c - c0 + 1) * 128].astype(BF16)))
                if extra is not None:
                    extra(c)

    blk0 = Blk(0, ZU + 1)
    b_copy.wait()
    bt = jnp.transpose(jnp.concatenate([b_ref[...].astype(F32)] * (128 * 128 // S), axis=0))
    for i in range(S // 128):
        btab_ref[i * 128:(i + 1) * 128, :] = jnp.broadcast_to(bt[:, i:i + 1], (128, 128))
    xa_copy.wait()
    xbs = [blk0.ln(i) for i in range(XA)]
    win0_copy.wait()
    for i in range(XA):
        blk0.z1_rows(i, xbs[i], c1=W0)
    win1_copy.wait()
    xb_copy.wait()
    for i in range(XA):
        blk0.z1_rows(i, xbs[i], c0=W0)
    for i in range(XA, ZU + 1):
        xbs.append(blk0.ln(i))
    blk0.z1_rows(XA, xbs[XA], c1=W1)
    win2_copy.wait()
    for i in ZORD0:
        blk0.z2_rows(i, xbs[i])
    blk0.z1_rows(XA, xbs[XA], c0=W1)
    xc_copy.wait()
    wq_copy(0).wait()

    def zgroup(c, carry):
        @pl.when(c == 2)
        def _():
            xd_copy.wait()
            wq_copy(1).wait()

        @pl.when(c == 3)
        def _():
            wq_copy(2).wait()

        blk = Blk(c * ZU, ZU)
        xbs = [_bf(blk.xn[:SB // 2, :])]
        for s in range(1, ZU):
            xbs.append(blk.ln(s))
        Blk(jnp.minimum((c + 1) * ZU, NB - 1), 1).ln(0)
        n1 = 0
        for kind, s in ZORD:
            if kind == 2:
                blk.z2_rows(s, xbs[s])
            else:
                def extra(t):
                    j0 = jnp.minimum((((c - 1) * ZU + n1) * (NT - 1) + t) * CJ, DH2 - CJ)
                    relayout(0, 0, j0, CJ)
                    relayout(0, 1, j0, CJ)
                blk.z1_rows(s, xbs[s], extra)
                n1 += 1
        return carry
    jax.lax.fori_loop(1, NZ, zgroup, 0)

    wk_copy.wait()
    UPP = NP // 4
    NJ = DH2 // UPP

    def qpre(i, carry):
        @pl.when(i * PG == NP // 2)
        def _():
            wv_copy.wait()

        xs = _bf(xs_ref[...])
        nr = NS // NCH
        nj = NJ // (2 * NCH)
        for k in range(PG):
            p = i * PG + k
            unit = p // UPP
            q = _dot(xs, wpair((0,), p))
            for par in range(2):
                for c in range(NCH):
                    wkv_ref[pl.ds(pl.multiple_of(QOFF + (2 * p + par) * NS + c * nr, 8), nr), :] = _pk(
                        q[c * nr:(c + 1) * nr, par * Dh:(par + 1) * Dh])
                    relayout(1 + unit // 2, unit % 2, (p % UPP) * NJ + (par * NCH + c) * nj, nj)
        return carry
    jax.lax.fori_loop(0, NP // PG, qpre, 0)

    def qpre_rows(p, r):
        return jnp.concatenate(
            [pltpu.bitcast(wkv_ref[pl.ds(pl.multiple_of(QOFF + (2 * p + par) * NS + r, 8), M), :], F32)
             for par in range(2)], axis=1)

    def gcol(jj, c):
        r0 = _mult(jj * R, R)
        g = _dot(wsp_ref[pl.ds(r0, R), :], _bf(z2_ref[:, c * 128:(c + 1) * 128])) + btab_ref[pl.ds(r0, R), :]
        z1 = _bf(wq_ref[pl.ds(_mult(ZOFF + c * (S // 2) + jj * SEG, 8), SEG), :]).astype(F32)
        return (_gelu(z1) * g).astype(BF16)

    def glast(it):
        r0 = _mult(it * RU, RU)
        gt = _dot_t(_bf(z2t_ref[:, :S]), wsp_ref[pl.ds(r0, RU), :])
        gt = jnp.concatenate([gt, jnp.zeros((128 - FP, RU), F32)], axis=0)
        g = jnp.transpose(gt)[:, :FP] + btab_ref[pl.ds(r0, RU), :FP]
        z1 = _bf(wq_ref[pl.ds(_mult(ZOFF + (NT - 1) * (S // 2) + it * R, 8), R), :FP]).astype(F32)
        return (_gelu(z1) * g).astype(BF16)

    wo_copy.wait()
    wout_copy.wait()
    mem0_copy.wait()
    wspa_copy.wait()
    for c in range(NCAR):
        tc_ref[:, c * 128:(c + 1) * 128] = _pk(gcol(0, c))

    scale = Dh ** -0.5
    c_exp = scale * math.log2(math.e)

    def main(it, mem):
        @pl.when(it == 1)
        def _():
            wspb_copy.wait()

        row = jax.lax.broadcasted_iota(jnp.int32, (2 * L, 2 * L), 0)
        col = jax.lax.broadcasted_iota(jnp.int32, (2 * L, 2 * L), 1)
        rhi = row >= L
        chi = col >= L
        rl = jnp.where(rhi, row - L, row)
        cl = jnp.where(chi, col - L, col)
        same = rhi == chi
        valid = same & ((rl < M) | (rl >= cl))
        fill = jnp.where(same, -1e9 / scale, -jnp.inf).astype(F32)

        def stack(a, i):
            return jnp.concatenate([a[:, i * Dh:(i + 1) * Dh], a[:, (i + 1) * Dh:(i + 2) * Dh]], axis=0).astype(BF16)

        def scores(q2, k2):
            s = jnp.where(valid, _dot_t(q2, k2), fill)
            m = jnp.max(s, axis=-1, keepdims=True)
            e = jnp.exp2((s - m) * c_exp)
            l = jnp.sum(e, axis=-1, keepdims=True)
            return e.astype(BF16), 1.0 / l

        def pv(e, inv_l, v2):
            o2 = _dot(e, v2) * inv_l
            return jnp.concatenate([o2[:L], o2[L:]], axis=1)

        def run_step(proj, pre_o, fillers):
            qkv, sm, oo = {}, {}, {}
            acc = None
            for t in range(NP + 3):
                if t < NP:
                    qkv[t] = proj(t)
                else:
                    fillers[t - NP]()
                p = t - 3
                if 0 <= p < NP:
                    tt = _dot(oo[p], wo_ref[p * 2 * Dh:(p + 1) * 2 * Dh, :])
                    acc = tt if acc is None else acc + tt
                p = t - 1
                if 0 <= p < NP:
                    sm[p] = scores(qkv[p][0], qkv[p][1])
                p = t - 2
                if 0 <= p < NP:
                    oo[p] = pre_o(p, pv(sm[p][0], sm[p][1], qkv[p][2])).astype(BF16)
            fillers[3]()
            return acc

        tl = []

        def pair_step(uu, mem, tcar):
            jj = it * UNR + uu
            r0 = pl.multiple_of(jj * R, R)
            q0 = jj * 2 * M
            xn = _bf(xn_ref[pl.ds(pl.multiple_of(jj * SEG, SEG), SEG), :]).astype(F32)
            jn = jnp.minimum(jj + 1, S // R - 1)
            tparts, tnext, gate = list(tcar), [], []

            def cur(c):
                return lambda: tparts.append(gcol(jj, c))

            def nxt(c):
                return lambda: tnext.append(gcol(jn, c))

            def gout(lo, hi):
                def f():
                    t = jnp.concatenate(tparts + [tl[0][uu * R:(uu + 1) * R]], axis=1)
                    u = _dot(t, wout_ref[:, lo:hi])
                    gate.append(u * jax.nn.sigmoid(u))
                return f

            def with_last(f):
                def g():
                    f()
                    if uu == 0:
                        tl.append(glast(it))
                return g

            stash_kv, stash_o = {}, {}

            hA = jnp.concatenate([mem, xn[:SEG + M]], axis=0).astype(BF16)

            def projA(p):
                q = _dot(hA[:SEG], wpair((0,), p))
                kv = _dot(hA, wpair((1, 2), p))
                stash_kv[p] = kv[L:]
                kv = kv[:L]
                q = jnp.concatenate([q, qpre_rows(p, q0)], axis=0)
                return stack(q, 0), stack(kv, 0), stack(kv, 2)

            def preA(p, o):
                stash_o[p] = o[SEG:]
                return o[:SEG]

            accA = run_step(projA, preA, [with_last(cur(2)), cur(3), cur(4), cur(5)])

            hB = jnp.concatenate([accA[:M], xn[SEG + M:]], axis=0).astype(BF16)

            def projB(p):
                r = _dot(hB, wpair((0, 1, 2), p))
                st = jnp.concatenate([qpre_rows(p, q0 + M), stash_kv[p]], axis=1)
                r = jnp.concatenate([r[:M], st, r[M:]], axis=0)
                return stack(r, 0), stack(r, 2), stack(r, 4)

            def preB(p, o):
                return jnp.concatenate([o, stash_o[p]], axis=0)

            accB = run_step(projB, preB, [gout(0, GS), nxt(0), gout(GS, D), nxt(1)])

            s_out = jnp.concatenate([accA[M:], accB[L:], accB[M:L]], axis=0)
            xr = x_ref[pl.ds(r0, R), :].astype(F32)
            o_ref[pl.ds(r0, R), :] = (xr + s_out * jnp.concatenate(gate, axis=1)).astype(o_ref.dtype)
            return accB[:M], tuple(tnext)

        tcar = tuple(_bf(tc_ref[:, c * 128:(c + 1) * 128]) for c in range(NCAR))
        for uu in range(UNR):
            mem, tcar = pair_step(uu, mem, tcar)
        out_copy(it).start()
        for c in range(NCAR):
            tc_ref[:, c * 128:(c + 1) * 128] = _pk(tcar[c])
        return mem

    jax.lax.fori_loop(0, NIT, main, mem0_ref[0].astype(F32))
    for i in range(NIT):
        out_copy(i).wait()


@functools.partial(jax.jit, static_argnames=("SEG",))
def _run(A_x, A_mem0, A_Wq, A_Wk, A_Wv, A_Wo, B_w_in, B_w_sp, B_b_sp, B_w_out, *, SEG):
    B, S, D = A_x.shape
    H, Dh = A_Wq.shape[1], A_Wq.shape[2]
    M = A_mem0.shape[1]
    FH = B_w_in.shape[1] // 2
    assert (B, S, D, H, Dh, M, SEG, FH) == (1, 2048, 640, 32, 128, 8, 32, 864)
    wq, wk, wv = (w.reshape(D * H, Dh) for w in (A_Wq, A_Wk, A_Wv))
    wo = A_Wo.reshape(H * Dh, D)
    b = B_b_sp.reshape(S // 128, 128)
    win_t = B_w_in.T
    NS = S // SEG * M
    RS = D // 2 + RPAD
    anyspec = pl.BlockSpec(memory_space=pl.ANY)
    return pl.pallas_call(
        functools.partial(_kernel, S=S, D=D, H=H, Dh=Dh, M=M, SEG=SEG, FH=FH),
        in_specs=[anyspec] * 10,
        out_specs=anyspec,
        out_shape=jax.ShapeDtypeStruct(A_x.shape, A_x.dtype),
        scratch_shapes=[
            pltpu.VMEM((S, D), BF16),
            pltpu.VMEM((S // 2, D), U32),
            pltpu.VMEM((NS // 2, D), U32),
            pltpu.VMEM((H * RS + -(-FH // 128) * (S // 2), Dh), U32),
            pltpu.VMEM((2 * H * RS + H * NS, Dh), U32),
            pltpu.VMEM((S // 2, FH // 128 * 128), U32),
            pltpu.VMEM((FH % 128 // 2, S + 128), U32),
            pltpu.VMEM(A_mem0.shape, BF16),
            pltpu.VMEM((3, D * H, Dh), BF16),
            pltpu.VMEM(wo.shape, BF16),
            pltpu.VMEM(win_t.shape, BF16),
            pltpu.VMEM(B_w_sp.shape, BF16),
            pltpu.VMEM(B_w_out.shape, BF16),
            pltpu.VMEM(b.shape, BF16),
            pltpu.VMEM((S, 128), F32),
            pltpu.VMEM((S, D), BF16),
            pltpu.VMEM((SEG, NCAR * 128), U32),
            pltpu.SemaphoreType.DMA((15 + S // (SB * ZU),)),
        ],
        compiler_params=pltpu.CompilerParams(vmem_limit_bytes=110 * 1024 * 1024),
    )(A_x, A_mem0, wq, wk, wv, wo, win_t, B_w_sp, b, B_w_out)


def pallas_recurrent_scan__memory_aug_recurrent_mem_tr__mixer_gmlp__prompt_kernel(
        A_x, A_mem0, A_Wq, A_Wk, A_Wv, A_Wo, A_seg_len, B_x, B_w_in, B_w_sp, B_b_sp, B_w_out):
    seg = A_seg_len if isinstance(A_seg_len, int) else 32
    return _run(A_x, A_mem0, A_Wq, A_Wk, A_Wv, A_Wo, B_w_in, B_w_sp, B_b_sp, B_w_out, SEG=seg)
```

```python
import functools
import math

import jax
import jax.numpy as jnp
import jax.experimental.pallas as pl
import jax.experimental.pallas.tpu as pltpu

F32 = jnp.float32
BF16 = jnp.bfloat16
U32 = jnp.uint32

RPAD = 4
UNR = 2
SB = 128
ZU = 4
PG = 8
NCH = 4
NCAR = 2
W1 = 3
GS = 256
W0 = 3
ZORD0 = (0, 3, 1, 2)
ZORD = [(1, 0), (1, 1), (1, 2), (2, 3), (2, 0), (2, 1), (2, 2), (1, 3)]
XA = 3


def _ln(x, eps=1e-5):
    m = jnp.mean(x, axis=-1, keepdims=True)
    xc = x - m
    v = jnp.mean(xc * xc, axis=-1, keepdims=True)
    return xc * jax.lax.rsqrt(v + eps)


def _dot(a, b):
    return jnp.dot(a, b, preferred_element_type=F32)


def _dot_t(a, b):
    return jax.lax.dot_general(a, b, (((1,), (1,)), ((), ())), preferred_element_type=F32)


def _bf(u):
    return pltpu.bitcast(u, BF16)


def _pk(x):
    return pltpu.bitcast(x, U32)


def _gelu(x):
    c0 = math.sqrt(2.0 / math.pi)
    u = x * (x * x * (c0 * 0.044715) + c0)
    h = 0.5 * x
    return h * jnp.tanh(u) + h


def _mult(i, k):
    return i if isinstance(i, int) else pl.multiple_of(i, k)


def _kernel(x_hbm, mem0_hbm, wq_hbm, wk_hbm, wv_hbm, wo_hbm, win_hbm, wsp_hbm, b_hbm, wout_hbm,
            o_hbm,
            x_ref, xn_ref, xs_ref, wq_ref, wkv_ref, z2_ref, z2t_ref, mem0_ref, wraw_ref, wo_ref, win_ref,
            wsp_ref, wout_ref, b_ref, btab_ref, o_ref, tc_ref, sems,
            *, S, D, H, Dh, M, SEG, FH):
    L = M + SEG
    R = 2 * SEG
    RU = R * UNR
    NIT = S // RU
    NP = H // 2
    HG = NP // 2
    DH2 = D // 2
    RS = DH2 + RPAD
    QL = SEG - M
    NS = S // R * 2 * M
    NX = SB // R * 2 * M
    NT = -(-FH // 128)
    FL = (NT - 1) * 128
    FP = FH - FL
    NB = S // SB
    NZ = NB // ZU
    ZOFF = H * RS
    QOFF = 2 * H * RS
    CJ = -(-DH2 // ((NZ - 1) * ZU * (NT - 1)))
    WQP = CJ * ZU * (NT - 1) * 2 * H

    sem_ids = iter(range(sems.shape[0]))

    def sem_block(n):
        return [next(sem_ids) for _ in range(n)][0]

    def rows_copy(src, dst, lo, n, sem):
        return pltpu.make_async_copy(src.at[pl.ds(lo, n), :], dst.at[pl.ds(lo, n), :], sems.at[sem])

    def full_copy(src, dst):
        return pltpu.make_async_copy(src, dst, sems.at[sem_block(1)])

    x2 = x_hbm.at[0]
    xa_copy = rows_copy(x2, x_ref, 0, XA * SB, sem_block(1))
    xb_copy = rows_copy(x2, x_ref, XA * SB, (ZU + 1 - XA) * SB, sem_block(1))
    xc_copy = rows_copy(x2, x_ref, (ZU + 1) * SB, ZU * SB, sem_block(1))
    xd_copy = rows_copy(x2, x_ref, (2 * ZU + 1) * SB, S - (2 * ZU + 1) * SB, sem_block(1))
    win0_copy = rows_copy(win_hbm, win_ref, 0, W0 * 128, sem_block(1))
    win1_copy = rows_copy(win_hbm, win_ref, W0 * 128, FH - W0 * 128, sem_block(1))
    win2_copy = rows_copy(win_hbm, win_ref, FH, FH, sem_block(1))
    wk_copy = full_copy(wk_hbm, wraw_ref.at[1])
    wv_copy = full_copy(wv_hbm, wraw_ref.at[2])
    wo_copy = full_copy(wo_hbm, wo_ref)
    wout_copy = full_copy(wout_hbm, wout_ref)
    mem0_copy = full_copy(mem0_hbm, mem0_ref)
    b_copy = full_copy(b_hbm, b_ref)
    wspa_copy = rows_copy(wsp_hbm, wsp_ref, 0, RU + R, sem_block(1))
    wspb_copy = rows_copy(wsp_hbm, wsp_ref, RU + R, S - RU - R, sem_block(1))
    wq_sem, out_sem = sem_block(NZ - 1), sem_block(1)

    def wq_copy(c):
        return rows_copy(wq_hbm, wraw_ref.at[0], c * WQP, min(WQP, D * H - c * WQP), wq_sem + c)

    def out_copy(i):
        return rows_copy(o_ref, o_hbm.at[0], i * RU, RU, out_sem)

    for c in ([b_copy, xa_copy, win0_copy, win1_copy, xb_copy, win2_copy, mem0_copy, xc_copy, wq_copy(0), xd_copy]
              + [wq_copy(c) for c in range(1, NZ - 1)] + [wk_copy, wv_copy, wo_copy, wout_copy, wspa_copy, wspb_copy]):
        c.start()

    def wdst(w):
        return (wq_ref, 0) if isinstance(w, int) and w == 0 else (wkv_ref, (w - 1) * H)

    def wpair(ws, p):
        parts = []
        for w in ws:
            ref, h0 = wdst(w)
            for par in range(2):
                parts.append(_bf(ref[pl.ds((h0 + par * NP + p) * RS, DH2), :]))
        return jnp.concatenate(parts, axis=1)

    def relayout(w, grp, j0, nj):
        src = wraw_ref.at[w, pl.ds(pl.multiple_of((j0 * H + grp * HG) * 2, HG * 2), (nj * H - HG) * 2), :]
        dst, h0 = wdst(w)
        base = (h0 + grp * HG) * RS + j0
        for u in range(nj):
            a = _pk(src[u * H * 2:(u * H + HG) * 2, :])
            b = _pk(src[(u * H + NP) * 2:(u * H + NP + HG) * 2, :])
            dst[pl.ds(base + u, HG, stride=RS), :] = (a & jnp.uint32(0xFFFF)) | (b << 16)
            dst[pl.ds(base + NP * RS + u, HG, stride=RS), :] = (a >> 16) | (b & jnp.uint32(0xFFFF0000))

    class Blk:
        def __init__(self, i0, n):
            v = lambda ref, k: ref.at[pl.ds(_mult(i0 * k, k), n * k), :]
            self.x, self.xn, self.xs, self.z2 = v(x_ref, SB), v(xn_ref, SB // 2), v(xs_ref, NX // 2), v(z2_ref, SB // 2)
            self.i0 = i0

        def ln(self, s):
            xn = _ln(self.x[s * SB:(s + 1) * SB, :].astype(F32))
            xb = xn.astype(BF16)
            self.xn[s * SB // 2:(s + 1) * SB // 2, :] = _pk(xb)
            sel = jnp.concatenate([xn[k * R + QL:k * R + QL + 2 * M] for k in range(SB // R)], axis=0)
            self.xs[s * NX // 2:(s + 1) * NX // 2, :] = _pk(sel.astype(BF16))
            return xb

        def z2_rows(self, s, xb):
            zt = _dot_t(jnp.concatenate([win_ref[FH + FL:, :], win_ref[FL:FH, :]], axis=0), xb)
            z1l = jnp.transpose(zt[FP:])
            wq_ref[pl.ds(_mult(ZOFF + (NT - 1) * (S // 2) + (self.i0 + s) * (SB // 2), 8), SB // 2), :FP] = (
                _pk(z1l.astype(BF16)))
            z2 = jnp.concatenate([_dot_t(xb, win_ref[FH:FH + FL, :]), jnp.transpose(zt[:FP])], axis=1)
            z2 = _ln(_gelu(z2))
            self.z2[s * SB // 2:(s + 1) * SB // 2, :] = _pk(z2[:, :FL].astype(BF16))
            z2t_ref[:, pl.ds(_mult((self.i0 + s) * SB, SB), SB)] = (
                _pk(jnp.transpose(z2[:, FL:]).astype(BF16)))

        def z1_rows(self, s, xb, extra=None, c0=0, c1=NT - 1):
            z1 = _dot_t(xb, win_ref[c0 * 128:c1 * 128, :])
            r = (self.i0 + s) * (SB // 2)
            for c in range(c0, c1):
                wq_ref[pl.ds(_mult(ZOFF + c * (S // 2) + r, 8), SB // 2), :] = (
                    _pk(z1[:, (c - c0) * 128:(c - c0 + 1) * 128].astype(BF16)))
                if extra is not None:
                    extra(c)

    blk0 = Blk(0, ZU + 1)
    b_copy.wait()
    bt = jnp.transpose(jnp.concatenate([b_ref[...].astype(F32)] * (128 * 128 // S), axis=0))
    for i in range(S // 128):
        btab_ref[i * 128:(i + 1) * 128, :] = jnp.broadcast_to(bt[:, i:i + 1], (128, 128))
    xa_copy.wait()
    xbs = [blk0.ln(i) for i in range(XA)]
    win0_copy.wait()
    for i in range(XA):
        blk0.z1_rows(i, xbs[i], c1=W0)
    win1_copy.wait()
    xb_copy.wait()
    for i in range(XA):
        blk0.z1_rows(i, xbs[i], c0=W0)
    for i in range(XA, ZU + 1):
        xbs.append(blk0.ln(i))
    blk0.z1_rows(XA, xbs[XA], c1=W1)
    win2_copy.wait()
    for i in ZORD0:
        blk0.z2_rows(i, xbs[i])
    blk0.z1_rows(XA, xbs[XA], c0=W1)
    xc_copy.wait()
    wq_copy(0).wait()

    def zgroup(c, carry):
        @pl.when(c == 2)
        def _():
            xd_copy.wait()
            wq_copy(1).wait()

        @pl.when(c == 3)
        def _():
            wq_copy(2).wait()

        blk = Blk(c * ZU, ZU)
        xbs = [_bf(blk.xn[:SB // 2, :])]
        for s in range(1, ZU):
            xbs.append(blk.ln(s))
        Blk(jnp.minimum((c + 1) * ZU, NB - 1), 1).ln(0)
        n1 = 0
        for kind, s in ZORD:
            if kind == 2:
                blk.z2_rows(s, xbs[s])
            else:
                def extra(t):
                    j0 = jnp.minimum((((c - 1) * ZU + n1) * (NT - 1) + t) * CJ, DH2 - CJ)
                    relayout(0, 0, j0, CJ)
                    relayout(0, 1, j0, CJ)
                blk.z1_rows(s, xbs[s], extra)
                n1 += 1
        return carry
    jax.lax.fori_loop(1, NZ, zgroup, 0)

    wk_copy.wait()
    UPP = NP // 4
    NJ = DH2 // UPP

    def qpre(i, carry):
        @pl.when(i * PG == NP // 2)
        def _():
            wv_copy.wait()

        xs = _bf(xs_ref[...])
        nr = NS // NCH
        nj = NJ // (2 * NCH)
        for k in range(PG):
            p = i * PG + k
            unit = p // UPP
            q = _dot(xs, wpair((0,), p))
            for par in range(2):
                for c in range(NCH):
                    wkv_ref[pl.ds(pl.multiple_of(QOFF + (2 * p + par) * NS + c * nr, 8), nr), :] = _pk(
                        q[c * nr:(c + 1) * nr, par * Dh:(par + 1) * Dh])
                    relayout(1 + unit // 2, unit % 2, (p % UPP) * NJ + (par * NCH + c) * nj, nj)
        return carry
    jax.lax.fori_loop(0, NP // PG, qpre, 0)

    def qpre_rows(p, r):
        return jnp.concatenate(
            [pltpu.bitcast(wkv_ref[pl.ds(pl.multiple_of(QOFF + (2 * p + par) * NS + r, 8), M), :], F32)
             for par in range(2)], axis=1)

    def gcol(jj, c):
        r0 = _mult(jj * R, R)
        g = _dot(wsp_ref[pl.ds(r0, R), :], _bf(z2_ref[:, c * 128:(c + 1) * 128])) + btab_ref[pl.ds(r0, R), :]
        z1 = _bf(wq_ref[pl.ds(_mult(ZOFF + c * (S // 2) + jj * SEG, 8), SEG), :]).astype(F32)
        return (_gelu(z1) * g).astype(BF16)

    def glast(it):
        r0 = _mult(it * RU, RU)
        gt = _dot_t(_bf(z2t_ref[:, :S]), wsp_ref[pl.ds(r0, RU), :])
        g = jnp.transpose(gt) + btab_ref[pl.ds(r0, RU), :FP]
        z1 = _bf(wq_ref[pl.ds(_mult(ZOFF + (NT - 1) * (S // 2) + it * R, 8), R), :FP]).astype(F32)
        return (_gelu(z1) * g).astype(BF16)

    wo_copy.wait()
    wout_copy.wait()
    mem0_copy.wait()
    wspa_copy.wait()
    for c in range(NCAR):
        tc_ref[:, c * 128:(c + 1) * 128] = _pk(gcol(0, c))

    scale = Dh ** -0.5
    c_exp = scale * math.log2(math.e)

    def main(it, mem):
        @pl.when(it == 1)
        def _():
            wspb_copy.wait()

        row = jax.lax.broadcasted_iota(jnp.int32, (2 * L, 2 * L), 0)
        col = jax.lax.broadcasted_iota(jnp.int32, (2 * L, 2 * L), 1)
        rhi = row >= L
        chi = col >= L
        rl = jnp.where(rhi, row - L, row)
        cl = jnp.where(chi, col - L, col)
        same = rhi == chi
        valid = same & ((rl < M) | (rl >= cl))
        fill = jnp.where(same, -1e9 / scale, -jnp.inf).astype(F32)

        def stack(a, i):
            return jnp.concatenate([a[:, i * Dh:(i + 1) * Dh], a[:, (i + 1) * Dh:(i + 2) * Dh]], axis=0).astype(BF16)

        def scores(q2, k2):
            s = jnp.where(valid, _dot_t(q2, k2), fill)
            m = jnp.max(s, axis=-1, keepdims=True)
            e = jnp.exp2((s - m) * c_exp)
            l = jnp.sum(e, axis=-1, keepdims=True)
            return e.astype(BF16), 1.0 / l

        def pv(e, inv_l, v2):
            o2 = _dot(e, v2) * inv_l
            return jnp.concatenate([o2[:L], o2[L:]], axis=1)

        def run_step(proj, pre_o, fillers):
            qkv, sm, oo = {}, {}, {}
            acc = None
            for t in range(NP + 3):
                if t < NP:
                    qkv[t] = proj(t)
                else:
                    fillers[t - NP]()
                p = t - 3
                if 0 <= p < NP:
                    tt = _dot(oo[p], wo_ref[p * 2 * Dh:(p + 1) * 2 * Dh, :])
                    acc = tt if acc is None else acc + tt
                p = t - 1
                if 0 <= p < NP:
                    sm[p] = scores(qkv[p][0], qkv[p][1])
                p = t - 2
                if 0 <= p < NP:
                    oo[p] = pre_o(p, pv(sm[p][0], sm[p][1], qkv[p][2])).astype(BF16)
            fillers[3]()
            return acc

        tl = []

        def pair_step(uu, mem, tcar):
            jj = it * UNR + uu
            r0 = pl.multiple_of(jj * R, R)
            q0 = jj * 2 * M
            xn = _bf(xn_ref[pl.ds(pl.multiple_of(jj * SEG, SEG), SEG), :]).astype(F32)
            jn = jnp.minimum(jj + 1, S // R - 1)
            tparts, tnext, gate = list(tcar), [], []

            def cur(c):
                return lambda: tparts.append(gcol(jj, c))

            def nxt(c):
                return lambda: tnext.append(gcol(jn, c))

            def gout(lo, hi):
                def f():
                    t = jnp.concatenate(tparts + [tl[0][uu * R:(uu + 1) * R]], axis=1)
                    u = _dot(t, wout_ref[:, lo:hi])
                    gate.append(u * jax.nn.sigmoid(u))
                return f

            def with_last(f):
                def g():
                    f()
                    if uu == 0:
                        tl.append(glast(it))
                return g

            stash_kv, stash_o = {}, {}

            hA = jnp.concatenate([mem, xn[:SEG + M]], axis=0).astype(BF16)

            def projA(p):
                q = _dot(hA[:SEG], wpair((0,), p))
                kv = _dot(hA, wpair((1, 2), p))
                stash_kv[p] = kv[L:]
                kv = kv[:L]
                q = jnp.concatenate([q, qpre_rows(p, q0)], axis=0)
                return stack(q, 0), stack(kv, 0), stack(kv, 2)

            def preA(p, o):
                stash_o[p] = o[SEG:]
                return o[:SEG]

            accA = run_step(projA, preA, [with_last(cur(2)), cur(3), cur(4), cur(5)])

            hB = jnp.concatenate([accA[:M], xn[SEG + M:]], axis=0).astype(BF16)

            def projB(p):
                r = _dot(hB, wpair((0, 1, 2), p))
                st = jnp.concatenate([qpre_rows(p, q0 + M), stash_kv[p]], axis=1)
                r = jnp.concatenate([r[:M], st, r[M:]], axis=0)
                return stack(r, 0), stack(r, 2), stack(r, 4)

            def preB(p, o):
                return jnp.concatenate([o, stash_o[p]], axis=0)

            accB = run_step(projB, preB, [gout(0, GS), nxt(0), gout(GS, D), nxt(1)])

            s_out = jnp.concatenate([accA[M:], accB[L:], accB[M:L]], axis=0)
            xr = x_ref[pl.ds(r0, R), :].astype(F32)
            o_ref[pl.ds(r0, R), :] = (xr + s_out * jnp.concatenate(gate, axis=1)).astype(o_ref.dtype)
            return accB[:M], tuple(tnext)

        tcar = tuple(_bf(tc_ref[:, c * 128:(c + 1) * 128]) for c in range(NCAR))
        for uu in range(UNR):
            mem, tcar = pair_step(uu, mem, tcar)
        out_copy(it).start()
        for c in range(NCAR):
            tc_ref[:, c * 128:(c + 1) * 128] = _pk(tcar[c])
        return mem

    jax.lax.fori_loop(0, NIT, main, mem0_ref[0].astype(F32))
    for i in range(NIT):
        out_copy(i).wait()


@functools.partial(jax.jit, static_argnames=("SEG",))
def _run(A_x, A_mem0, A_Wq, A_Wk, A_Wv, A_Wo, B_w_in, B_w_sp, B_b_sp, B_w_out, *, SEG):
    B, S, D = A_x.shape
    H, Dh = A_Wq.shape[1], A_Wq.shape[2]
    M = A_mem0.shape[1]
    FH = B_w_in.shape[1] // 2
    assert (B, S, D, H, Dh, M, SEG, FH) == (1, 2048, 640, 32, 128, 8, 32, 864)
    wq, wk, wv = (w.reshape(D * H, Dh) for w in (A_Wq, A_Wk, A_Wv))
    wo = A_Wo.reshape(H * Dh, D)
    b = B_b_sp.reshape(S // 128, 128)
    win_t = B_w_in.T
    NS = S // SEG * M
    RS = D // 2 + RPAD
    anyspec = pl.BlockSpec(memory_space=pl.ANY)
    return pl.pallas_call(
        functools.partial(_kernel, S=S, D=D, H=H, Dh=Dh, M=M, SEG=SEG, FH=FH),
        in_specs=[anyspec] * 10,
        out_specs=anyspec,
        out_shape=jax.ShapeDtypeStruct(A_x.shape, A_x.dtype),
        scratch_shapes=[
            pltpu.VMEM((S, D), BF16),
            pltpu.VMEM((S // 2, D), U32),
            pltpu.VMEM((NS // 2, D), U32),
            pltpu.VMEM((H * RS + -(-FH // 128) * (S // 2), Dh), U32),
            pltpu.VMEM((2 * H * RS + H * NS, Dh), U32),
            pltpu.VMEM((S // 2, FH // 128 * 128), U32),
            pltpu.VMEM((FH % 128 // 2, S + 128), U32),
            pltpu.VMEM(A_mem0.shape, BF16),
            pltpu.VMEM((3, D * H, Dh), BF16),
            pltpu.VMEM(wo.shape, BF16),
            pltpu.VMEM(win_t.shape, BF16),
            pltpu.VMEM(B_w_sp.shape, BF16),
            pltpu.VMEM(B_w_out.shape, BF16),
            pltpu.VMEM(b.shape, BF16),
            pltpu.VMEM((S, 128), F32),
            pltpu.VMEM((S, D), BF16),
            pltpu.VMEM((SEG, NCAR * 128), U32),
            pltpu.SemaphoreType.DMA((15 + S // (SB * ZU),)),
        ],
        compiler_params=pltpu.CompilerParams(vmem_limit_bytes=110 * 1024 * 1024),
    )(A_x, A_mem0, wq, wk, wv, wo, win_t, B_w_sp, b, B_w_out)


def pallas_recurrent_scan__memory_aug_recurrent_mem_tr__mixer_gmlp__prompt_kernel(
        A_x, A_mem0, A_Wq, A_Wk, A_Wv, A_Wo, A_seg_len, B_x, B_w_in, B_w_sp, B_b_sp, B_w_out):
    seg = A_seg_len if isinstance(A_seg_len, int) else 32
    return _run(A_x, A_mem0, A_Wq, A_Wk, A_Wv, A_Wo, B_w_in, B_w_sp, B_b_sp, B_w_out, SEG=seg)
```
